```python
import os as _os
_os.environ.setdefault("JAX_PLATFORMS", "cpu")
import jax
import jax.numpy as jnp

def _softmax(x, axis=-1):
    return jax.nn.softmax(x, axis=axis)
def _gelu(x):
    return jax.nn.gelu(x, approximate=True)
def _silu(x):
    return jax.nn.silu(x)
def _sigmoid(x):
    return jax.nn.sigmoid(x)
def _layernorm(x, axis=-1, eps=1e-5):
    m = jnp.mean(x, axis=axis, keepdims=True)
    v = jnp.var(x, axis=axis, keepdims=True)
    return (x - m) / jnp.sqrt(v + eps)
def _scatter_add(tgt, idx, src, axis=0):
    return tgt.at[idx].add(src)
def _segment_sum(src, seg, n):
    return jax.ops.segment_sum(src, seg, n)
class _Rng:
    def __init__(self, key):
        self._k = key
    def _next(self):
        self._k, sub = jax.random.split(self._k)
        return sub
    def normal(self, shape):
        return jax.random.normal(self._next(), shape, dtype=jnp.bfloat16)
    def randint(self, lo, hi, shape):
        return jax.random.randint(self._next(), shape, lo, hi, dtype=jnp.int32)
    def uniform(self, shape, lo=0.0, hi=1.0):
        return jax.random.uniform(self._next(), shape, jnp.bfloat16, lo, hi)
    def permutation(self, n):
        return jax.random.permutation(self._next(), n)


kernel_name = 'parallel_sum__mha_block__swiglu_ffn__prompt'

def setup_inputs():
    _rng = _Rng(jax.random.key(int.from_bytes(__import__("os").urandom(4), "little")))
    _w = (lambda a: (lambda t: t.astype(jnp.bfloat16) if jnp.issubdtype(t.dtype, jnp.floating) else t)(jnp.asarray(a)))
    def _A_setup():
        B, S, D, H = 1, 2048, 640, 32
        return {
            "x": _w((lambda *s: _rng.normal(s) * 0.05)(B, S, D)),
            "wqkv": _w((lambda *s: _rng.normal(s) * 0.1)(D, 3 * D)),
            "wo": _w((lambda *s: _rng.normal(s) * 0.05)(D, D)),
        }
    _A_in = _A_setup()

    def _B_setup():
        B, S, D, F = 1, 2048, 640, 1536
        return {
            "x": _w((lambda *s: _rng.normal(s) * 0.05)(B, S, D)),
            "w_gate": _w((lambda *s: _rng.normal(s) * 0.05)(D, F)),
            "w_up": _w((lambda *s: _rng.normal(s) * 0.05)(D, F)),
            "w_down": _w((lambda *s: _rng.normal(s) * 0.05)(F, D)),
        }
    _B_in = _B_setup()

    return {
        "A_x": _A_in["x"],
        "A_wqkv": _A_in["wqkv"],
        "A_wo": _A_in["wo"],
        "B_x": _B_in["x"],
        "B_w_gate": _B_in["w_gate"],
        "B_w_up": _B_in["w_up"],
        "B_w_down": _B_in["w_down"],
    }

def reference(A_x, A_wqkv, A_wo, B_x, B_w_gate, B_w_up, B_w_down):
    def _A_ref(x, wqkv, wo):
        B, S, D = x.shape
        H = 32
        Dh = D // H
        qkv = (lambda x, *d: x.transpose(*d))((x @ wqkv).reshape(B, S, 3, H, Dh), 2, 0, 3, 1, 4)
        q, k, v = qkv[0], qkv[1], qkv[2]
        scores = jnp.einsum("bhqd,bhkd->bhqk", q, k) * (Dh ** -0.5)
        p = _softmax(scores, axis=-1)
        o = jnp.einsum("bhqk,bhkd->bhqd", p, v)
        return (lambda x, *d: x.transpose(*d))(o, 0, 2, 1, 3).reshape(B, S, D) @ wo

    def _B_ref(x, w_gate, w_up, w_down):
        g = _silu(x @ w_gate)
        u = x @ w_up
        return (g * u) @ w_down

    x = A_x
    xn = _layernorm(x, axis=-1)
    return x + _A_ref(xn, A_wqkv, A_wo) + _B_ref(xn, B_w_gate, B_w_up, B_w_down)
```

```python
import functools
import math

import jax
import jax.numpy as jnp
from jax import lax
import jax.experimental.pallas as pl
import jax.experimental.pallas.tpu as pltpu

S, D, H, DH, F = 2048, 640, 32, 20, 1536
HPG = 6
NG = -(-H // HPG)
GW = HPG * DH
QSCALE = (DH ** -0.5) * math.log2(math.e)
M_OFFSET = 64.0
L_MIN = 2.0 ** -60
ACC_MAX = 2.0 ** 120

f32 = jnp.float32
bf16 = jnp.bfloat16
NT = (((1,), (1,)), ((), ()))
TN = (((0,), (0,)), ((), ()))


def make_kernel(TQ=512, KC=256, PC=512, FC=512, DEPTH=2, TR=512, FORCE_FALLBACK=False):
    NQ = S // TQ
    NPC = S // PC
    NR = S // TR

    def kernel(x_hbm, wqkv_hbm, wo_hbm, wg_hbm, wu_hbm, wd_hbm, o_hbm,
               x_ref, wqkv_ref, wo_ref, wg_ref, wu_ref, wd_ref, ob_ref,
               xn_ref, k_ref, qm_ref, qt_ref, vt_ref, wqvt_ref, wk_ref, kn2_ref, ot_ref,
               sem_x, sem_w, sem_o):
        x_cp = [pltpu.make_async_copy(x_hbm.at[c * PC:(c + 1) * PC], x_ref.at[c * PC:(c + 1) * PC],
                                      sem_x.at[c]) for c in range(NPC)]
        wk_cp = pltpu.make_async_copy(wqkv_hbm.at[:, D:2 * D + 128], wqkv_ref.at[:, D:2 * D + 128],
                                      sem_w.at[0])
        wq_cp = pltpu.make_async_copy(wqkv_hbm.at[:, 0:D], wqkv_ref.at[:, 0:D], sem_w.at[1])
        wv_cp = pltpu.make_async_copy(wqkv_hbm.at[:, 2 * D + 128:3 * D],
                                      wqkv_ref.at[:, 2 * D + 128:3 * D], sem_w.at[2])
        late_cp = [pltpu.make_async_copy(s, d, sem_w.at[3 + i]) for i, (s, d) in enumerate(
            [(wo_hbm, wo_ref), (wg_hbm, wg_ref), (wu_hbm, wu_ref), (wd_hbm, wd_ref)])]
        x_cp[0].start()
        wk_cp.start()
        for c in range(1, NPC):
            x_cp[c].start()
        wq_cp.start()
        wv_cp.start()

        def layernorm(c):
            x = x_ref[c * PC:(c + 1) * PC, :].astype(f32)
            mu = jnp.mean(x, axis=-1, keepdims=True)
            xc = x - mu
            var = jnp.mean(xc * xc, axis=-1, keepdims=True)
            xn_ref[c * PC:(c + 1) * PC, :] = (xc * lax.rsqrt(var + 1e-5)).astype(bf16)

        lane = lax.broadcasted_iota(jnp.int32, (PC, 128), 1)
        er = lax.broadcasted_iota(jnp.int32, (H, 128), 0)
        ec = lax.broadcasted_iota(jnp.int32, (H, 128), 1)

        def kproj(c):
            xn = xn_ref[c * PC:(c + 1) * PC, :]
            kall = jnp.dot(xn, wk_ref[...], preferred_element_type=f32)
            kn2 = None
            for g in range(NG):
                nvalid = min(GW, D - GW * g)
                kg = kall[:, g * 128:(g + 1) * 128]
                kf = jnp.where(lane < nvalid, kg, 0.0).astype(bf16).astype(f32)
                e = ((ec >= (er - HPG * g) * DH) & (ec < (er - HPG * g) * DH + DH)
                     & (er >= HPG * g) & (er < HPG * g + HPG))
                e = jnp.where(e, 1.0, 0.0).astype(bf16)
                t = lax.dot_general(e, (kf * kf).astype(bf16), NT, preferred_element_type=f32)
                kn2 = t if kn2 is None else kn2 + t
                k_ref[g, c * PC:(c + 1) * PC, :] = jnp.where(
                    (lane >= GW) & (lane < GW + 3), 1.0, kf).astype(bf16)
            kn2_ref[:, c * PC:(c + 1) * PC] = kn2

        x_cp[0].wait()
        layernorm(0)
        wk_cp.wait()
        for g in range(NG):
            wk_ref[:, g * 128:(g + 1) * 128] = wqkv_ref[:, D + GW * g: D + GW * g + 128]
        for c in range(NPC):
            if c + 1 < NPC:
                x_cp[c + 1].wait()
                layernorm(c + 1)
            else:
                wq_cp.wait()
                wv_cp.wait()
                for cp in late_cp:
                    cp.start()
                wqvt_ref[0:D, :] = wqkv_ref[:, 0:D].astype(f32).T.astype(bf16)
                wqvt_ref[D:2 * D, :] = wqkv_ref[:, 2 * D:3 * D].astype(f32).T.astype(bf16)
            kproj(c)

        kmax2 = jnp.max(kn2_ref[...], axis=-1, keepdims=True)

        er2 = lax.broadcasted_iota(jnp.int32, (H, D), 0)
        ec2 = lax.broadcasted_iota(jnp.int32, (H, D), 1)
        e2 = jnp.where((ec2 >= er2 * DH) & (ec2 < er2 * DH + DH), 1.0, 0.0).astype(bf16)
        rows16 = lax.broadcasted_iota(jnp.int32, (16, PC), 0)
        sub_pc = lax.broadcasted_iota(jnp.int32, (8, PC), 0)

        def qv(c, carry):
            r0 = pl.multiple_of(c * PC, PC)
            xn = xn_ref[pl.ds(r0, PC), :]
            qt = lax.dot_general(wqvt_ref[0:D, :], xn, NT, preferred_element_type=f32)
            qt = (qt * QSCALE).astype(bf16).astype(f32)
            qn2 = jnp.dot(e2, (qt * qt).astype(bf16), preferred_element_type=f32)
            vt = lax.dot_general(wqvt_ref[D:2 * D, :], xn, NT, preferred_element_type=f32)
            negm = M_OFFSET - jnp.sqrt(qn2 * kmax2) * (1.0 + 2.0 ** -6)
            zero16 = jnp.zeros((16, PC), bf16)
            for h in range(H):
                g, j = h // HPG, h % HPG
                lo, hi = DH * j, DH * j + DH
                for r in range(7):
                    a, b = 16 * r, 16 * r + 16
                    if b <= lo or a >= hi:
                        blk = zero16
                    else:
                        src0 = GW * g + a
                        win = qt[src0:src0 + 16] if src0 + 16 <= D else jnp.concatenate(
                            [qt[src0:D], jnp.zeros((src0 + 16 - D, PC), f32)], axis=0)
                        if a >= lo and b <= hi:
                            blk = win.astype(bf16)
                        else:
                            blk = jnp.where((rows16 >= lo - a) & (rows16 < hi - a), win,
                                            0.0).astype(bf16)
                    qm_ref[h, a:b, pl.ds(r0, PC)] = blk
                qt_ref[h, 0:8, pl.ds(r0, PC)] = (
                    qt[GW * g + 112:GW * g + 120] if j == HPG - 1 else jnp.zeros((8, PC), f32))
                qt_ref[h, 8:16, pl.ds(r0, PC)] = jnp.where(sub_pc == 0, negm[h:h + 1, :], 0.0)
                w0 = 8 * ((DH * h) // 8)
                vw = jnp.concatenate([vt[w0:w0 + 24], jnp.ones((8, PC), f32)], axis=0)
                vt_ref[h, :, pl.ds(r0, PC)] = vw.astype(bf16)
            return carry

        lax.fori_loop(0, NPC, qv, 0)

        sub = lax.broadcasted_iota(jnp.int32, (8, TQ), 0)

        def load_qm(h, q0):
            return jnp.concatenate([qm_ref[h, :, pl.ds(q0, TQ)],
                                    qt_ref[h, :, pl.ds(q0, TQ)].astype(bf16)], axis=0)

        def attn_step(it, bad):
            p = it // NQ
            q0 = pl.multiple_of((it % NQ) * TQ, TQ)
            hs = [2 * p, 2 * p + 1]
            qms = [load_qm(h, q0) for h in hs]
            gs = [h // HPG for h in hs]
            accs = [None, None]
            steps = [(i, c) for i in range(2) for c in range(S // KC)]

            def qk(step):
                i, c = step
                st = jnp.dot(k_ref[gs[i], c * KC:(c + 1) * KC, :], qms[i],
                             preferred_element_type=f32)
                return jnp.exp2(st).astype(bf16)

            pts = [qk(s) for s in steps[:DEPTH]]
            for n, (i, c) in enumerate(steps):
                if n + DEPTH < len(steps):
                    pts.append(qk(steps[n + DEPTH]))
                pv = jnp.dot(vt_ref[hs[i], :, c * KC:(c + 1) * KC], pts[n],
                             preferred_element_type=f32)
                accs[i] = pv if accs[i] is None else accs[i] + pv

            outs = []
            for a in accs:
                l = a[24:32]
                r = 1.0 / l
                amax = jnp.maximum(jnp.maximum(jnp.abs(a[0:8]), jnp.abs(a[8:16])),
                                   jnp.maximum(jnp.abs(a[16:24]), l))
                ok = (l >= L_MIN) & (amax <= ACC_MAX)
                bad = jnp.where(ok, bad, 1.0)
                outs.append([a[0:8] * r, a[8:16] * r, a[16:24] * r])
            mid = jnp.where(sub < 4, outs[0][2], outs[1][0])
            o = jnp.concatenate([outs[0][0], outs[0][1], mid, outs[1][1], outs[1][2]], axis=0)
            ot_ref[pl.ds(pl.multiple_of(p * 40, 8), 40), pl.ds(q0, TQ)] = o
            return bad

        def attention():
            return lax.fori_loop(0, (H // 2) * NQ, attn_step, jnp.zeros((8, TQ), f32))

        bad = attention()
        unsafe = jnp.max(bad) > 0.0
        if FORCE_FALLBACK:
            unsafe = jnp.max(bad) > -1.0

        @pl.when(unsafe)
        def _fallback():
            def true_max(it, carry):
                h = it // NQ
                q0 = pl.multiple_of((it % NQ) * TQ, TQ)
                qt_ref[h, 8:16, pl.ds(q0, TQ)] = jnp.zeros((8, TQ), f32)
                qm = load_qm(h, q0)
                g = h // HPG

                def chunk(c, mx):
                    st = jnp.dot(k_ref[g, pl.ds(pl.multiple_of(c * KC, KC), KC), :], qm,
                                 preferred_element_type=f32)
                    return jnp.maximum(mx, jnp.max(st, axis=0, keepdims=True))

                mx = lax.fori_loop(0, S // KC, chunk, jnp.full((1, TQ), -jnp.inf, f32))
                m1 = mx.astype(bf16).astype(f32)
                m2 = (mx - m1).astype(bf16).astype(f32)
                m3 = (mx - m1 - m2).astype(bf16).astype(f32)
                qt_ref[h, 8:16, pl.ds(q0, TQ)] = jnp.where(
                    sub == 0, -m1, jnp.where(sub == 1, -m2, jnp.where(sub == 2, -m3, 0.0)))
                return carry

            lax.fori_loop(0, H * NQ, true_max, 0)
            attention()

        for cp in late_cp:
            cp.wait()

        def out_copy(t, slot):
            return pltpu.make_async_copy(ob_ref.at[slot],
                                         o_hbm.at[pl.ds(pl.multiple_of(t * TR, TR), TR)],
                                         sem_o.at[slot])

        def tail(t, carry):
            r0 = pl.multiple_of(t * TR, TR)
            slot = t % 2
            xn = xn_ref[pl.ds(r0, TR), :]
            y = x_ref[pl.ds(r0, TR), :].astype(f32)
            y = y + lax.dot_general(ot_ref[:, pl.ds(r0, TR)].astype(bf16), wo_ref[...], TN,
                                    preferred_element_type=f32)
            for c in range(F // FC):
                g = jnp.dot(xn, wg_ref[:, c * FC:(c + 1) * FC], preferred_element_type=f32)
                u = jnp.dot(xn, wu_ref[:, c * FC:(c + 1) * FC], preferred_element_type=f32)
                hh = (g * jax.nn.sigmoid(g) * u).astype(bf16)
                y = y + jnp.dot(hh, wd_ref[c * FC:(c + 1) * FC, :], preferred_element_type=f32)

            @pl.when(t >= 2)
            def _():
                out_copy(t - 2, slot).wait()

            ob_ref[slot] = y.astype(bf16)
            out_copy(t, slot).start()
            return carry

        lax.fori_loop(0, NR, tail, 0)
        for t in range(max(NR - 2, 0), NR):
            out_copy(t, t % 2).wait()

    def run(A_x, A_wqkv, A_wo, B_x, B_w_gate, B_w_up, B_w_down):
        x = A_x.reshape(S, D)
        anyspec = pl.BlockSpec(memory_space=pl.ANY)
        out = pl.pallas_call(
            kernel,
            in_specs=[anyspec] * 6,
            out_specs=anyspec,
            out_shape=jax.ShapeDtypeStruct((S, D), bf16),
            scratch_shapes=[
                pltpu.VMEM((S, D), bf16),
                pltpu.VMEM((D, 3 * D), bf16),
                pltpu.VMEM((D, D), bf16),
                pltpu.VMEM((D, F), bf16),
                pltpu.VMEM((D, F), bf16),
                pltpu.VMEM((F, D), bf16),
                pltpu.VMEM((2, TR, D), bf16),
                pltpu.VMEM((S, D), bf16),
                pltpu.VMEM((NG, S, 128), bf16),
                pltpu.VMEM((H, 112, S), bf16),
                pltpu.VMEM((H, 16, S), f32),
                pltpu.VMEM((H, 32, S), bf16),
                pltpu.VMEM((2 * D, D), bf16),
                pltpu.VMEM((D, NG * 128), bf16),
                pltpu.VMEM((H, S), f32),
                pltpu.VMEM((D, S), f32),
                pltpu.SemaphoreType.DMA((NPC,)),
                pltpu.SemaphoreType.DMA((7,)),
                pltpu.SemaphoreType.DMA((2,)),
            ],
            compiler_params=pltpu.CompilerParams(vmem_limit_bytes=110 * 1024 * 1024),
        )(x, A_wqkv, A_wo, B_w_gate, B_w_up, B_w_down)
        return out.reshape(1, S, D)

    return run


_run = make_kernel()


@jax.jit
def pallas_parallel_sum__mha_block__swiglu_ffn__prompt_kernel(
    A_x: jax.Array,
    A_wqkv: jax.Array,
    A_wo: jax.Array,
    B_x: jax.Array,
    B_w_gate: jax.Array,
    B_w_up: jax.Array,
    B_w_down: jax.Array,
):
    return _run(A_x, A_wqkv, A_wo, B_x, B_w_gate, B_w_up, B_w_down)
```

```python
import functools
import math

import jax
import jax.numpy as jnp
from jax import lax
import jax.experimental.pallas as pl
import jax.experimental.pallas.tpu as pltpu

S, D, H, DH, F = 2048, 640, 32, 20, 1536
HPG = 6
NG = -(-H // HPG)
GW = HPG * DH
QSCALE = (DH ** -0.5) * math.log2(math.e)
M_OFFSET = 64.0
L_MIN = 2.0 ** -60
ACC_MAX = 2.0 ** 120

f32 = jnp.float32
bf16 = jnp.bfloat16
NT = (((1,), (1,)), ((), ()))
TN = (((0,), (0,)), ((), ()))
NN = (((1,), (0,)), ((), ()))


def make_kernel(TQ=512, KC=256, PC=512, FC=512, DEPTH=2, TR=256, FORCE_FALLBACK=False, N1=None, N2=None, N3=None, NOCHECK=False, PMEM=True, NPB=8):
    NQ = S // TQ
    NPC = S // PC
    NR = S // TR

    def kernel(x_hbm, wqkv_hbm, wo_hbm, wg_hbm, wu_hbm, wd_hbm, o_hbm,
               x_ref, wqkv_ref, wo_ref, wg_ref, wu_ref, wd_ref, ob_ref,
               xn_ref, k_ref, qt_ref, sh_ref, vt_ref, wqvt_ref, wk_ref, kn2_ref, ot_ref, p_ref, xv_ref,
               sem_x, sem_w, sem_o):
        x_cp = [pltpu.make_async_copy(x_hbm.at[c * PC:(c + 1) * PC], x_ref.at[c * PC:(c + 1) * PC],
                                      sem_x.at[c]) for c in range(NPC)]
        wk_cp = pltpu.make_async_copy(wqkv_hbm.at[:, D:2 * D + 128], wqkv_ref.at[:, D:2 * D + 128],
                                      sem_w.at[0])
        wq_cp = pltpu.make_async_copy(wqkv_hbm.at[:, 0:D], wqkv_ref.at[:, 0:D], sem_w.at[1])
        wv_cp = pltpu.make_async_copy(wqkv_hbm.at[:, 2 * D + 128:3 * D],
                                      wqkv_ref.at[:, 2 * D + 128:3 * D], sem_w.at[2])
        late_cp = [pltpu.make_async_copy(s, d, sem_w.at[3 + i]) for i, (s, d) in enumerate(
            [(wo_hbm, wo_ref), (wg_hbm, wg_ref), (wu_hbm, wu_ref), (wd_hbm, wd_ref)])]
        x_cp[0].start()
        wk_cp.start()
        for c in range(1, NPC):
            x_cp[c].start()
        wq_cp.start()
        wv_cp.start()

        def layernorm(c):
            x = x_ref[c * PC:(c + 1) * PC, :].astype(f32)
            mu = jnp.mean(x, axis=-1, keepdims=True)
            xc = x - mu
            var = jnp.mean(xc * xc, axis=-1, keepdims=True)
            xnf = xc * lax.rsqrt(var + 1e-5)
            xn_ref[c * PC:(c + 1) * PC, :] = xnf.astype(bf16)
            e = xnf.reshape(PC // 16, 2, 8, D)
            xv_ref[c * PC // 2:(c + 1) * PC // 2, :] = pltpu.pack_elementwise(
                [e[:, 0].reshape(PC // 2, D), e[:, 1].reshape(PC // 2, D)], packed_dtype=bf16)

        lane = lax.broadcasted_iota(jnp.int32, (PC, 128), 1)
        er = lax.broadcasted_iota(jnp.int32, (H, 128), 0)
        ec = lax.broadcasted_iota(jnp.int32, (H, 128), 1)

        def kproj(c):
            xn = xn_ref[c * PC:(c + 1) * PC, :]
            kall = jnp.dot(xn, wk_ref[...], preferred_element_type=f32)
            kn2 = None
            for g in range(NG):
                nvalid = min(GW, D - GW * g)
                kg = kall[:, g * 128:(g + 1) * 128]
                kf = jnp.where(lane < nvalid, kg, 0.0).astype(bf16).astype(f32)
                e = ((ec >= (er - HPG * g) * DH) & (ec < (er - HPG * g) * DH + DH)
                     & (er >= HPG * g) & (er < HPG * g + HPG))
                e = jnp.where(e, 1.0, 0.0).astype(bf16)
                t = lax.dot_general(e, (kf * kf).astype(bf16), NT, preferred_element_type=f32)
                kn2 = t if kn2 is None else kn2 + t
                k_ref[g, c * PC:(c + 1) * PC, :] = jnp.where(
                    (lane >= GW) & (lane < GW + 3), 1.0, kf).astype(bf16)
            kn2_ref[:, c * PC:(c + 1) * PC] = kn2

        x_cp[0].wait()
        layernorm(0)
        wk_cp.wait()
        for g in range(NG):
            wk_ref[:, g * 128:(g + 1) * 128] = wqkv_ref[:, D + GW * g: D + GW * g + 128]
        for c in range(NPC):
            if c + 1 < NPC:
                x_cp[c + 1].wait()
                layernorm(c + 1)
            else:
                wq_cp.wait()
                wv_cp.wait()
                for cp in late_cp:
                    cp.start()
                wqvt_ref[0:D, :] = wqkv_ref[:, 0:D].astype(f32).T.astype(bf16)
                wqvt_ref[D:2 * D, :] = wqkv_ref[:, 2 * D:3 * D].astype(f32).T.astype(bf16)
            kproj(c)

        kmax2 = jnp.max(kn2_ref[...], axis=-1, keepdims=True)

        er2 = lax.broadcasted_iota(jnp.int32, (H, D), 0)
        ec2 = lax.broadcasted_iota(jnp.int32, (H, D), 1)
        e2 = jnp.where((ec2 >= er2 * DH) & (ec2 < er2 * DH + DH), 1.0, 0.0).astype(bf16)
        sub_pc = lax.broadcasted_iota(jnp.int32, (8, PC), 0)

        def qv(c, carry):
            r0 = pl.multiple_of(c * PC, PC)
            xn = xn_ref[pl.ds(r0, PC), :]
            qt = lax.dot_general(wqvt_ref[0:D, :], xn, NT, preferred_element_type=f32)
            qt = (qt * QSCALE).astype(bf16).astype(f32)
            qt_ref[:, pl.ds(r0, PC)] = qt
            qn2 = jnp.dot(e2, (qt * qt).astype(bf16), preferred_element_type=f32)
            xv = pltpu.bitcast(xv_ref[pl.ds(pl.multiple_of(c * (PC // 2), PC // 2), PC // 2), :], bf16)
            vt = lax.dot_general(wqvt_ref[D:2 * D, :], xv, NT, preferred_element_type=f32)
            negm = M_OFFSET - jnp.sqrt(qn2 * kmax2) * (1.0 + 2.0 ** -6)
            for h in range(H):
                sh_ref[h, :, pl.ds(r0, PC)] = jnp.where(sub_pc == 0, negm[h:h + 1, :], 0.0)
                w0 = 8 * ((DH * h) // 8)
                if h % 2 == 0:
                    vw = jnp.concatenate(
                        [vt[w0:w0 + 16], jnp.where(sub_pc < 4, vt[w0 + 16:w0 + 24], 1.0)], axis=0)
                else:
                    vw = jnp.concatenate(
                        [jnp.where(sub_pc >= 4, vt[w0:w0 + 8], 1.0), vt[w0 + 8:w0 + 24]], axis=0)
                vt_ref[h, :, pl.ds(r0, PC)] = vw
            return carry

        lax.fori_loop(0, NPC, qv, 0)

        sub = lax.broadcasted_iota(jnp.int32, (8, TQ), 0)

        def load_qm(g, j, q0):
            lo, hi = DH * j, DH * j + DH
            base = pl.multiple_of(g * GW, 8)
            rows = []
            for r in range(15):
                a, b = 8 * r, 8 * r + 8
                if b <= lo or a >= hi:
                    rows.append(None)
                    continue
                v = qt_ref[pl.ds(base + a, 8), pl.ds(q0, TQ)]
                if a < lo:
                    v = jnp.where(sub >= lo - a, v, 0.0)
                elif b > hi:
                    v = jnp.where(sub < hi - a, v, 0.0)
                rows.append(v)
            rows.append(sh_ref[g * HPG + j, :, pl.ds(q0, TQ)])
            blocks = []
            for r in range(8):
                a, b = rows[2 * r], rows[2 * r + 1]
                if a is None and b is None:
                    blocks.append(jnp.zeros((16, TQ), bf16))
                else:
                    a = jnp.zeros((8, TQ), f32) if a is None else a
                    b = jnp.zeros((8, TQ), f32) if b is None else b
                    blocks.append(jnp.concatenate([a, b], axis=0).astype(bf16))
            return jnp.concatenate(blocks, axis=0)

        def attn_group(g, tq, nh, bad):
            q0 = pl.multiple_of(tq * TQ, TQ)
            qms = [None] * nh
            accs = [None] * nh
            cnt = [0]
            steps = [(j, c) for j in range(nh) for c in range(S // KC)]

            def qk(j, c):
                if qms[j] is None:
                    qms[j] = load_qm(g, j, q0)
                st = jnp.dot(k_ref[g, c * KC:(c + 1) * KC, :], qms[j], preferred_element_type=f32)
                if not PMEM:
                    return jnp.exp2(st).astype(bf16)
                slot = cnt[0] % NPB
                cnt[0] += 1
                e = jnp.exp2(st).reshape(KC // 16, 2, 8, TQ)
                p_ref[slot] = pltpu.pack_elementwise(
                    [e[:, 0].reshape(KC // 2, TQ), e[:, 1].reshape(KC // 2, TQ)], packed_dtype=bf16)
                return slot

            def finish(j, bad):
                outs = []
                for odd, a in enumerate((accs[j], accs[j + 1])):
                    lv = a[0:8] if odd else a[16:24]
                    keep = (sub < 4) if odd else (sub >= 4)
                    l = jnp.where(keep, lv, pltpu.roll(lv, 4, 0))
                    r = 1.0 / l
                    amax = jnp.maximum(jnp.maximum(jnp.abs(a[0:8]), jnp.abs(a[8:16])),
                                       jnp.abs(a[16:24]))
                    ok = (l >= L_MIN) & (amax <= ACC_MAX)
                    bad = jnp.where(ok, bad, 1.0)
                    outs.append([a[0:8] * r, a[8:16] * r, a[16:24] * r])
                mid = jnp.where(sub < 4, outs[0][2], outs[1][0])
                o = jnp.concatenate([outs[0][0], outs[0][1], mid, outs[1][1], outs[1][2]], axis=0)
                ot_ref[pl.ds(pl.multiple_of(g * GW + j * DH, 8), 40), pl.ds(q0, TQ)] = o
                return bad

            pts = [qk(*s) for s in steps[:DEPTH]]
            for n, (j, c) in enumerate(steps):
                if n + DEPTH < len(steps):
                    pts.append(qk(*steps[n + DEPTH]))
                ptn = pts[n] if not PMEM else pltpu.bitcast(p_ref[pts[n]], bf16)
                pv = lax.dot_general(vt_ref[g * HPG + j, :, c * KC:(c + 1) * KC], ptn, NN,
                                     preferred_element_type=f32)
                pts[n] = None
                accs[j] = pv if accs[j] is None else accs[j] + pv
                if j % 2 == 1 and c == S // KC - 1:
                    bad = finish(j - 1, bad)
            return bad

        NFULL = H // HPG

        def attention():
            bad = lax.fori_loop(
                0, NFULL * NQ if N1 is None else N1, lambda it, bad: attn_group(it // NQ, it % NQ, HPG, bad),
                jnp.zeros((8, TQ), f32))
            return lax.fori_loop(
                0, NQ if N2 is None else N2, lambda it, bad: attn_group(NFULL, it, H - NFULL * HPG, bad), bad)

        def true_max():
            rows128 = lax.broadcasted_iota(jnp.int32, (128, TQ), 0)

            def one(it, carry):
                h = it // NQ
                q0 = pl.multiple_of((it % NQ) * TQ, TQ)
                g = h // HPG
                lo = (h % HPG) * DH
                base = pl.multiple_of(jnp.minimum(g * GW, D - 128), 8)
                win = qt_ref[pl.ds(base, 128), pl.ds(q0, TQ)]
                win = pltpu.roll(win, (128 - (g * GW - base)) % 128, 0)
                qm = jnp.where((rows128 >= lo) & (rows128 < lo + DH), win, 0.0).astype(bf16)

                def chunk(c, mx):
                    st = jnp.dot(k_ref[g, pl.ds(pl.multiple_of(c * 256, 256), 256), :], qm,
                                 preferred_element_type=f32)
                    return jnp.maximum(mx, jnp.max(st, axis=0, keepdims=True))

                mx = lax.fori_loop(0, S // 256, chunk, jnp.full((1, TQ), -jnp.inf, f32))
                m1 = mx.astype(bf16).astype(f32)
                m2 = (mx - m1).astype(bf16).astype(f32)
                m3 = (mx - m1 - m2).astype(bf16).astype(f32)
                sh_ref[h, :, pl.ds(q0, TQ)] = jnp.where(
                    sub == 0, -m1, jnp.where(sub == 1, -m2, jnp.where(sub == 2, -m3, 0.0)))
                return carry

            lax.fori_loop(0, H * NQ, one, 0)

        def attempt(state):
            n, _ = state

            @pl.when(n > 0)
            def _():
                true_max()

            bad = attention()
            unsafe = jnp.max(bad) > (-1.0 if FORCE_FALLBACK else (5.0 if NOCHECK else 0.0))
            return n + 1, unsafe.astype(jnp.int32)

        lax.while_loop(lambda s: (s[0] < 2) & (s[1] > 0), attempt,
                       (jnp.int32(0), jnp.int32(1)))

        for cp in late_cp:
            cp.wait()

        def out_copy(t, slot):
            return pltpu.make_async_copy(ob_ref.at[slot],
                                         o_hbm.at[pl.ds(pl.multiple_of(t * TR, TR), TR)],
                                         sem_o.at[slot])

        def tail(t, carry):
            r0 = pl.multiple_of(t * TR, TR)
            slot = t % 2

            @pl.when(t >= 2)
            def _():
                out_copy(t - 2, slot).wait()

            xn = xn_ref[pl.ds(r0, TR), :]
            y = x_ref[pl.ds(r0, TR), :].astype(f32)
            for c in range(F // FC):
                g = jnp.dot(xn, wg_ref[:, c * FC:(c + 1) * FC], preferred_element_type=f32)
                u = jnp.dot(xn, wu_ref[:, c * FC:(c + 1) * FC], preferred_element_type=f32)
                if c == F // FC - 1:
                    y = y + lax.dot_general(ot_ref[:, pl.ds(r0, TR)].astype(bf16), wo_ref[...], TN,
                                            preferred_element_type=f32)
                hh = (g * jax.nn.sigmoid(g) * u).astype(bf16)
                y = y + jnp.dot(hh, wd_ref[c * FC:(c + 1) * FC, :], preferred_element_type=f32)
            ob_ref[slot] = y.astype(bf16)
            out_copy(t, slot).start()
            return carry

        lax.fori_loop(0, NR, tail, 0)
        for t in range(max(NR - 2, 0), NR):
            out_copy(t, t % 2).wait()

    def run(A_x, A_wqkv, A_wo, B_x, B_w_gate, B_w_up, B_w_down):
        x = A_x.reshape(S, D)
        anyspec = pl.BlockSpec(memory_space=pl.ANY)
        out = pl.pallas_call(
            kernel,
            in_specs=[anyspec] * 6,
            out_specs=anyspec,
            out_shape=jax.ShapeDtypeStruct((S, D), bf16),
            scratch_shapes=[
                pltpu.VMEM((S, D), bf16),
                pltpu.VMEM((D, 3 * D), bf16),
                pltpu.VMEM((D, D), bf16),
                pltpu.VMEM((D, F), bf16),
                pltpu.VMEM((D, F), bf16),
                pltpu.VMEM((F, D), bf16),
                pltpu.VMEM((2, TR, D), bf16),
                pltpu.VMEM((S, D), bf16),
                pltpu.VMEM((NG, S, 128), bf16),
                pltpu.VMEM((D, S), f32),
                pltpu.VMEM((H, 8, S), f32),
                pltpu.VMEM((H, 24, S), f32),
                pltpu.VMEM((2 * D, D), bf16),
                pltpu.VMEM((D, NG * 128), bf16),
                pltpu.VMEM((H, S), f32),
                pltpu.VMEM((D, S), f32),
                pltpu.VMEM((NPB, KC // 2, TQ), jnp.uint32),
                pltpu.VMEM((S // 2, D), jnp.uint32),
                pltpu.SemaphoreType.DMA((NPC,)),
                pltpu.SemaphoreType.DMA((7,)),
                pltpu.SemaphoreType.DMA((2,)),
            ],
            compiler_params=pltpu.CompilerParams(vmem_limit_bytes=110 * 1024 * 1024),
        )(x, A_wqkv, A_wo, B_w_gate, B_w_up, B_w_down)
        return out.reshape(1, S, D)

    return run


_run = make_kernel()


@jax.jit
def pallas_parallel_sum__mha_block__swiglu_ffn__prompt_kernel(
    A_x: jax.Array,
    A_wqkv: jax.Array,
    A_wo: jax.Array,
    B_x: jax.Array,
    B_w_gate: jax.Array,
    B_w_up: jax.Array,
    B_w_down: jax.Array,
):
    return _run(A_x, A_wqkv, A_wo, B_x, B_w_gate, B_w_up, B_w_down)
```

```python
import math

import jax
import jax.numpy as jnp
from jax import lax
import jax.experimental.pallas as pl
import jax.experimental.pallas.tpu as pltpu

S, D, H, DH, F = 2048, 640, 32, 20, 1536
HPG = 4
NG = H // HPG
GW = HPG * DH
QSCALE = (DH ** -0.5) * math.log2(math.e)
M_OFFSET = 72.0
L_MIN = 2.0 ** -40
ACC_MAX = 2.0 ** 120

f32 = jnp.float32
bf16 = jnp.bfloat16
NT = (((1,), (1,)), ((), ()))
TN = (((0,), (0,)), ((), ()))
NN = (((1,), (0,)), ((), ()))


def make_kernel(TQ=512, KC=128, PC=512, DEPTH=6, TR=256, FC=512, NPB=8, GPI=2,
                KCH=(512, 512, 512, 512), MS=128, ILV=False,
                FORCE_FALLBACK=False, NOCHECK=False, N1=None, EARLY=False, NSPLIT=True):
    NQ = S // TQ
    NPC = S // PC
    NR = S // TR
    koff = [sum(KCH[:i]) for i in range(len(KCH) + 1)]
    assert koff[-1] == S
    NK = len(KCH)

    def interleave_pack(v):
        n, m = v.shape
        e = v.reshape(n // 16, 2, 8, m)
        return pltpu.pack_elementwise(
            [e[:, 0].reshape(n // 2, m), e[:, 1].reshape(n // 2, m)], packed_dtype=bf16)

    def kernel(x_hbm, wqkv_hbm, wo_hbm, wg_hbm, wu_hbm, wd_hbm, o_hbm,
               x_ref, wqkv_ref, wo_ref, wg_ref, wu_ref, wd_ref, ob_ref,
               xn_ref, xv_ref, k_ref, qt_ref, sh_ref, vt_ref, wqvt_ref, kn2_ref, ot_ref, p_ref,
               sem_x, sem_w, sem_o):
        x_cp = [pltpu.make_async_copy(x_hbm.at[koff[c]:koff[c + 1]], x_ref.at[koff[c]:koff[c + 1]],
                                      sem_x.at[c]) for c in range(NK)]
        wk_cp, wq_cp, wv_cp = [
            pltpu.make_async_copy(wqkv_hbm.at[:, a:a + D], wqkv_ref.at[:, a:a + D], sem_w.at[i])
            for i, a in enumerate((D, 0, 2 * D))]
        late_cp = [pltpu.make_async_copy(s, d, sem_w.at[3 + i]) for i, (s, d) in enumerate(
            [(wo_hbm, wo_ref), (wg_hbm, wg_ref), (wu_hbm, wu_ref), (wd_hbm, wd_ref)])]
        x_cp[0].start()
        wk_cp.start()
        for c in range(1, NK):
            x_cp[c].start()
        wq_cp.start()
        wv_cp.start()

        def layernorm(c):
            a, b = koff[c], koff[c + 1]
            x = x_ref[a:b, :].astype(f32)
            mu = jnp.mean(x, axis=-1, keepdims=True)
            xc = x - mu
            var = jnp.mean(xc * xc, axis=-1, keepdims=True)
            xnf = xc * lax.rsqrt(var + 1e-5)
            xn_ref[a:b, :] = xnf.astype(bf16)
            if ILV:
                xv_ref[a // 2:b // 2, :] = interleave_pack(xnf)

        er2 = lax.broadcasted_iota(jnp.int32, (H, D), 0)
        ec2 = lax.broadcasted_iota(jnp.int32, (H, D), 1)
        e2f = jnp.where((ec2 >= er2 * DH) & (ec2 < er2 * DH + DH), 1.0, 0.0)
        e2 = e2f.astype(bf16)

        def head_sums(sq, transposed):
            if not NSPLIT:
                return lax.dot_general(e2, sq, NT if transposed else NN, preferred_element_type=f32)
            out = []
            for b in range(H // 8):
                lo = (8 * DH * b) // 128 * 128
                hi = -(-(8 * DH * (b + 1)) // 128) * 128
                w = sq[:, lo:hi] if transposed else sq[lo:hi, :]
                out.append(lax.dot_general(e2f[8 * b:8 * b + 8, lo:hi], w, NT if transposed else NN,
                                           preferred_element_type=f32))
            return jnp.concatenate(out, axis=0)

        def kproj(c):
            a, b = koff[c], koff[c + 1]
            n = b - a
            lane = lax.broadcasted_iota(jnp.int32, (n, 128 - GW), 1)
            kconst = jnp.where(lane < 3, 1.0, 0.0)
            kall = jnp.concatenate([
                jnp.dot(xn_ref[m:m + MS, :], wqkv_ref[:, D:2 * D], preferred_element_type=f32)
                for m in range(a, b, MS)], axis=0)
            kn2_ref[:, a:b] = head_sums((kall * kall).astype(bf16), True)
            for g in range(NG):
                k_ref[g, a:b, :] = jnp.concatenate(
                    [kall[:, g * GW:(g + 1) * GW], kconst], axis=1).astype(bf16)

        x_cp[0].wait()
        layernorm(0)
        wk_cp.wait()
        if EARLY:
            kproj(0)
            x_cp[1].wait()
            layernorm(1)
        else:
            x_cp[1].wait()
            kproj(0)
            layernorm(1)
        for c in range(2, NK):
            x_cp[c].wait()
        for c in range(1, NK - 1):
            kproj(c)
            layernorm(c + 1)
        wq_cp.wait()
        wv_cp.wait()
        for cp in late_cp:
            cp.start()
        kproj(NK - 1)
        wqvt_ref[0:D, :] = wqkv_ref[:, 0:D].astype(f32).T.astype(bf16)
        wqvt_ref[D:2 * D, :] = wqkv_ref[:, 2 * D:3 * D].astype(f32).T.astype(bf16)

        kmax2 = jnp.max(kn2_ref[...], axis=-1, keepdims=True)

        sub_pc = lax.broadcasted_iota(jnp.int32, (8, PC), 0)

        def qv(c, carry):
            r0 = pl.multiple_of(c * PC, PC)
            xn = xn_ref[pl.ds(r0, PC), :]
            qt = lax.dot_general(wqvt_ref[0:D, :], xn, NT, preferred_element_type=f32)
            qt = (qt * QSCALE).astype(bf16).astype(f32)
            qt_ref[:, pl.ds(r0, PC)] = qt
            qn2 = head_sums((qt * qt).astype(bf16), False)
            if ILV:
                xv = pltpu.bitcast(
                    xv_ref[pl.ds(pl.multiple_of(c * (PC // 2), PC // 2), PC // 2), :], bf16)
            else:
                xv = xn
            vt = lax.dot_general(wqvt_ref[D:2 * D, :], xv, NT, preferred_element_type=f32)
            negm = M_OFFSET - jnp.sqrt(qn2 * kmax2) * (1.0 + 2.0 ** -6)
            for h in range(H):
                sh_ref[h, :, pl.ds(r0, PC)] = jnp.where(sub_pc == 0, negm[h:h + 1, :], 0.0)
                w0 = 8 * ((DH * h) // 8)
                if h % 2 == 0:
                    vw = jnp.concatenate(
                        [vt[w0:w0 + 16], jnp.where(sub_pc < 4, vt[w0 + 16:w0 + 24], 1.0)], axis=0)
                else:
                    vw = jnp.concatenate(
                        [jnp.where(sub_pc >= 4, vt[w0:w0 + 8], 1.0), vt[w0 + 8:w0 + 24]], axis=0)
                vt_ref[h, :, pl.ds(r0, PC)] = vw
            return carry

        lax.fori_loop(0, NPC, qv, 0)

        sub = lax.broadcasted_iota(jnp.int32, (8, TQ), 0)

        def load_qm(g, j, q0):
            lo, hi = DH * j, DH * j + DH
            base = pl.multiple_of(g * GW, 8)
            rows = []
            for r in range(GW // 8):
                a, b = 8 * r, 8 * r + 8
                if b <= lo or a >= hi:
                    rows.append(None)
                    continue
                v = qt_ref[pl.ds(base + a, 8), pl.ds(q0, TQ)]
                if a < lo:
                    v = jnp.where(sub >= lo - a, v, 0.0)
                elif b > hi:
                    v = jnp.where(sub < hi - a, v, 0.0)
                rows.append(v)
            rows.append(sh_ref[g * HPG + j, :, pl.ds(q0, TQ)])
            rows += [None] * (16 - len(rows))
            blocks = []
            for r in range(8):
                a, b = rows[2 * r], rows[2 * r + 1]
                if a is None and b is None:
                    blocks.append(jnp.zeros((16, TQ), bf16))
                else:
                    a = jnp.zeros((8, TQ), f32) if a is None else a
                    b = jnp.zeros((8, TQ), f32) if b is None else b
                    blocks.append(jnp.concatenate([a, b], axis=0).astype(bf16))
            return jnp.concatenate(blocks, axis=0)

        def attn_step(it, bad):
            g0 = (it // NQ) * GPI
            q0 = pl.multiple_of((it % NQ) * TQ, TQ)
            nh = GPI * HPG
            qms = [None] * nh
            accs = [None] * nh
            nc = S // KC
            steps = [(i, c) for i in range(nh) for c in range(nc)]

            def qk(n):
                i, c = steps[n]
                g = g0 + i // HPG
                if qms[i] is None:
                    qms[i] = load_qm(g, i % HPG, q0)
                st = jnp.dot(k_ref[g, c * KC:(c + 1) * KC, :], qms[i], preferred_element_type=f32)
                if ILV:
                    p_ref[n % NPB] = interleave_pack(jnp.exp2(st))
                else:
                    p_ref[n % NPB] = jnp.exp2(st).astype(bf16)

            def finish(i, bad):
                outs = []
                for odd, a in enumerate((accs[i], accs[i + 1])):
                    lv = a[0:8] if odd else a[16:24]
                    keep = (sub < 4) if odd else (sub >= 4)
                    l = jnp.where(keep, lv, pltpu.roll(lv, 4, 0))
                    r = 1.0 / l
                    amax = jnp.maximum(jnp.maximum(jnp.abs(a[0:8]), jnp.abs(a[8:16])),
                                       jnp.abs(a[16:24]))
                    ok = (l >= L_MIN) & (amax <= ACC_MAX)
                    bad = jnp.where(ok, bad, 1.0)
                    outs.append([a[0:8] * r, a[8:16] * r, a[16:24] * r])
                mid = jnp.where(sub < 4, outs[0][2], outs[1][0])
                o = jnp.concatenate([outs[0][0], outs[0][1], mid, outs[1][1], outs[1][2]], axis=0)
                ot_ref[pl.ds(pl.multiple_of(g0 * GW + i * DH, 8), 40), pl.ds(q0, TQ)] = o
                return bad

            for n in range(DEPTH):
                qk(n)
            for n, (i, c) in enumerate(steps):
                if n + DEPTH < len(steps):
                    qk(n + DEPTH)
                pt = pltpu.bitcast(p_ref[n % NPB], bf16) if ILV else p_ref[n % NPB]
                pv = lax.dot_general(vt_ref[g0 * HPG + i, :, c * KC:(c + 1) * KC], pt, NN,
                                     preferred_element_type=f32)
                accs[i] = pv if accs[i] is None else accs[i] + pv
                if i % 2 == 1 and c == nc - 1:
                    bad = finish(i - 1, bad)
            return bad

        def true_max():
            rows80 = lax.broadcasted_iota(jnp.int32, (GW, TQ), 0)

            def one(it, carry):
                h = it // NQ
                q0 = pl.multiple_of((it % NQ) * TQ, TQ)
                g = h // HPG
                lo = (h % HPG) * DH
                win = qt_ref[pl.ds(pl.multiple_of(g * GW, 8), GW), pl.ds(q0, TQ)]
                qm = jnp.concatenate(
                    [jnp.where((rows80 >= lo) & (rows80 < lo + DH), win, 0.0),
                     jnp.zeros((128 - GW, TQ), f32)], axis=0).astype(bf16)

                def chunk(c, mx):
                    st = jnp.dot(k_ref[g, pl.ds(pl.multiple_of(c * 256, 256), 256), :], qm,
                                 preferred_element_type=f32)
                    return jnp.maximum(mx, jnp.max(st, axis=0, keepdims=True))

                mx = lax.fori_loop(0, S // 256, chunk, jnp.full((1, TQ), -jnp.inf, f32))
                m1 = mx.astype(bf16).astype(f32)
                m2 = (mx - m1).astype(bf16).astype(f32)
                m3 = (mx - m1 - m2).astype(bf16).astype(f32)
                sh_ref[h, :, pl.ds(q0, TQ)] = jnp.where(
                    sub == 0, -m1, jnp.where(sub == 1, -m2, jnp.where(sub == 2, -m3, 0.0)))
                return carry

            lax.fori_loop(0, H * NQ, one, 0)

        def attempt(state):
            n, _ = state

            @pl.when(n > 0)
            def _():
                true_max()

            bad = lax.fori_loop(0, (NG // GPI) * NQ if N1 is None else N1, attn_step,
                                jnp.zeros((8, TQ), f32))
            unsafe = jnp.max(bad) > (-1.0 if FORCE_FALLBACK else (5.0 if NOCHECK else 0.0))
            return n + 1, unsafe.astype(jnp.int32)

        lax.while_loop(lambda s: (s[0] < 2) & (s[1] > 0), attempt,
                       (jnp.int32(0), jnp.int32(1)))

        for cp in late_cp:
            cp.wait()

        def out_copy(t, slot):
            return pltpu.make_async_copy(ob_ref.at[slot],
                                         o_hbm.at[pl.ds(pl.multiple_of(t * TR, TR), TR)],
                                         sem_o.at[slot])

        def tail(t, carry):
            r0 = pl.multiple_of(t * TR, TR)
            slot = t % 2

            @pl.when(t >= 2)
            def _():
                out_copy(t - 2, slot).wait()

            xn = xn_ref[pl.ds(r0, TR), :]
            y = x_ref[pl.ds(r0, TR), :].astype(f32)
            for c in range(F // FC):
                g = jnp.dot(xn, wg_ref[:, c * FC:(c + 1) * FC], preferred_element_type=f32)
                u = jnp.dot(xn, wu_ref[:, c * FC:(c + 1) * FC], preferred_element_type=f32)
                if c == F // FC - 1:
                    y = y + lax.dot_general(ot_ref[:, pl.ds(r0, TR)].astype(bf16), wo_ref[...], TN,
                                            preferred_element_type=f32)
                hh = (g * jax.nn.sigmoid(g) * u).astype(bf16)
                y = y + jnp.dot(hh, wd_ref[c * FC:(c + 1) * FC, :], preferred_element_type=f32)
            ob_ref[slot] = y.astype(bf16)
            out_copy(t, slot).start()
            return carry

        lax.fori_loop(0, NR, tail, 0)
        for t in range(max(NR - 2, 0), NR):
            out_copy(t, t % 2).wait()

    def run(A_x, A_wqkv, A_wo, B_x, B_w_gate, B_w_up, B_w_down):
        x = A_x.reshape(S, D)
        anyspec = pl.BlockSpec(memory_space=pl.ANY)
        out = pl.pallas_call(
            kernel,
            in_specs=[anyspec] * 6,
            out_specs=anyspec,
            out_shape=jax.ShapeDtypeStruct((S, D), bf16),
            scratch_shapes=[
                pltpu.VMEM((S, D), bf16),
                pltpu.VMEM((D, 3 * D), bf16),
                pltpu.VMEM((D, D), bf16),
                pltpu.VMEM((D, F), bf16),
                pltpu.VMEM((D, F), bf16),
                pltpu.VMEM((F, D), bf16),
                pltpu.VMEM((2, TR, D), bf16),
                pltpu.VMEM((S, D), bf16),
                pltpu.VMEM((S // 2 if ILV else 8, D), jnp.uint32),
                pltpu.VMEM((NG, S, 128), bf16),
                pltpu.VMEM((D, S), f32),
                pltpu.VMEM((H, 8, S), f32),
                pltpu.VMEM((H, 24, S), f32),
                pltpu.VMEM((2 * D, D), bf16),
                pltpu.VMEM((H, S), f32),
                pltpu.VMEM((D, S), f32),
                (pltpu.VMEM((NPB, KC // 2, TQ), jnp.uint32) if ILV
                 else pltpu.VMEM((NPB, KC, TQ), bf16)),
                pltpu.SemaphoreType.DMA((NK,)),
                pltpu.SemaphoreType.DMA((7,)),
                pltpu.SemaphoreType.DMA((2,)),
            ],
            compiler_params=pltpu.CompilerParams(vmem_limit_bytes=110 * 1024 * 1024),
        )(x, A_wqkv, A_wo, B_w_gate, B_w_up, B_w_down)
        return out.reshape(1, S, D)

    return run


_run = make_kernel(NSPLIT=False)


@jax.jit
def pallas_parallel_sum__mha_block__swiglu_ffn__prompt_kernel(
    A_x: jax.Array,
    A_wqkv: jax.Array,
    A_wo: jax.Array,
    B_x: jax.Array,
    B_w_gate: jax.Array,
    B_w_up: jax.Array,
    B_w_down: jax.Array,
):
    return _run(A_x, A_wqkv, A_wo, B_x, B_w_gate, B_w_up, B_w_down)
```

```python
import math

import jax
import jax.numpy as jnp
from jax import lax
import jax.experimental.pallas as pl
import jax.experimental.pallas.tpu as pltpu

S, D, H, DH, F = 2048, 640, 32, 20, 1536
HPG = 4
NG = H // HPG
GW = HPG * DH
GPI = 2
NH = GPI * HPG
NI = NG // GPI
QSCALE = (DH ** -0.5) * math.log2(math.e)
M_OFFSET = 72.0
L_MIN = 2.0 ** -40
ACC_MAX = 2.0 ** 120

f32 = jnp.float32
bf16 = jnp.bfloat16
u32 = jnp.uint32
NT = (((1,), (1,)), ((), ()))
TN = (((0,), (0,)), ((), ()))
NN = (((1,), (0,)), ((), ()))


def make_kernel(KC=256, PC=512, DEPTH=3, TR=256, FC=512, NPB=8, MS=128, KV=128, XP=5,
                FORCE_FALLBACK=False, NOCHECK=False, N1=None, PTIE=True, TO=256, PDYN=True):
    TQ = 512
    NT128 = TQ // 128
    NQ = S // TQ
    NPC = S // PC
    NR = S // TR
    KCH = (512, 512, 512, 512)
    koff = [sum(KCH[:i]) for i in range(len(KCH) + 1)]
    NK = len(KCH)
    KM = S - KV
    KL = -(-KV // 128) * 128
    mchunks = [(c, min(c + KC, S - KL)) for c in range(0, S - KL, KC)]
    if KL > KV:
        mchunks.append((S - KL, KM))
    assert NQ == 4 and NI == 4 and KV % 16 == 0 and DH % XP == 0

    def interleave_pack(v):
        n, m = v.shape
        e = v.reshape(n // 16, 2, 8, m)
        return pltpu.pack_elementwise(
            [e[:, 0].reshape(n // 2, m), e[:, 1].reshape(n // 2, m)], packed_dtype=bf16)

    def kernel(x_hbm, wqkv_hbm, wo_hbm, wg_hbm, wu_hbm, wd_hbm, o_hbm,
               x_ref, wqkv_ref, wo_ref, wg_ref, wu_ref, wd_ref, ob_ref,
               xn_ref, xv_ref, k_ref, qt_ref, sh_ref, vt_ref, wqvt_ref, kn2_ref, ot_ref,
               pl_ref, kf_ref, kb_ref, y_ref,
               sem_x, sem_w, sem_o, z_ref, *pbuf):
        z_ref[0] = 0
        x_cp = [pltpu.make_async_copy(x_hbm.at[koff[c]:koff[c + 1]], x_ref.at[koff[c]:koff[c + 1]],
                                      sem_x.at[c]) for c in range(NK)]
        wk_cp, wq_cp, wv_cp = [
            pltpu.make_async_copy(wqkv_hbm.at[:, a:a + D], wqkv_ref.at[:, a:a + D], sem_w.at[i])
            for i, a in enumerate((D, 0, 2 * D))]
        late_cp = [pltpu.make_async_copy(s, d, sem_w.at[3 + i]) for i, (s, d) in enumerate(
            [(wo_hbm, wo_ref), (wg_hbm, wg_ref), (wu_hbm, wu_ref), (wd_hbm, wd_ref)])]
        x_cp[0].start()
        wk_cp.start()
        for c in range(1, NK):
            x_cp[c].start()
        wq_cp.start()
        wv_cp.start()

        def layernorm(c):
            a, b = koff[c], koff[c + 1]
            x = x_ref[a:b, :].astype(f32)
            mu = jnp.mean(x, axis=-1, keepdims=True)
            xc = x - mu
            var = jnp.mean(xc * xc, axis=-1, keepdims=True)
            xnf = xc * lax.rsqrt(var + 1e-5)
            xn_ref[a:b, :] = xnf.astype(bf16)
            xv_ref[a // 2:b // 2, :] = interleave_pack(xnf)

        er2 = lax.broadcasted_iota(jnp.int32, (H, D), 0)
        ec2 = lax.broadcasted_iota(jnp.int32, (H, D), 1)
        e2 = jnp.where((ec2 >= er2 * DH) & (ec2 < er2 * DH + DH), 1.0, 0.0).astype(bf16)

        def kproj(c):
            a, b = koff[c], koff[c + 1]
            n = b - a
            lane = lax.broadcasted_iota(jnp.int32, (n, 128 - GW), 1)
            kconst = jnp.where(lane < 3, 1.0, 0.0)
            kall = jnp.concatenate([
                jnp.dot(xn_ref[m:m + MS, :], wqkv_ref[:, D:2 * D], preferred_element_type=f32)
                for m in range(a, b, MS)], axis=0)
            kn2_ref[:, a:b] = lax.dot_general(e2, (kall * kall).astype(bf16), NT,
                                              preferred_element_type=f32)
            for g in range(NG):
                k_ref[g, a:b, :] = jnp.concatenate(
                    [kall[:, g * GW:(g + 1) * GW], kconst], axis=1).astype(bf16)
            if KV and b == S:
                kv = kall[n - KV:, :].astype(bf16).astype(f32)
                for pr in range(H // 2):
                    blk = jnp.concatenate([kv[:, 2 * DH * pr:2 * DH * (pr + 1)],
                                           jnp.zeros((KV, 128 - 2 * DH), f32)], axis=1)
                    kf_ref[0, pr] = blk
                    kf_ref[1, pr] = blk

        x_cp[0].wait()
        layernorm(0)
        wk_cp.wait()
        x_cp[1].wait()
        kproj(0)
        layernorm(1)
        for c in range(2, NK):
            x_cp[c].wait()
        for c in range(1, NK - 1):
            kproj(c)
            layernorm(c + 1)
        wq_cp.wait()
        wv_cp.wait()
        for cp in late_cp:
            cp.start()
        kproj(NK - 1)
        wqvt_ref[0:D, :] = wqkv_ref[:, 0:D].astype(f32).T.astype(bf16)
        wqvt_ref[D:2 * D, :] = wqkv_ref[:, 2 * D:3 * D].astype(f32).T.astype(bf16)

        kmax2 = jnp.max(kn2_ref[...], axis=-1, keepdims=True)

        def kf_rows(pr, r0, tie):
            if tie is None:
                return kf_ref[0, pr, pl.ds(r0, 8), :]
            return jnp.where(tie > 0.0, kf_ref[0, pr, pl.ds(r0, 8), :], kf_ref[1, pr, pl.ds(r0, 8), :])

        def bcast(kk, f):
            return jnp.broadcast_to(kk[:, f:f + 1], (8, 128))

        def make_kb(pairs, ties, nties):
            jobs = [(pr, u, f0) for pr in pairs for u in range(KV // 8)
                    for f0 in range(0, 2 * DH, 2 * XP)]
            for n, (pr, u, f0) in enumerate(jobs):
                kk = kf_rows(pr, 8 * u, ties(n * nties // len(jobs)) if PTIE else None)
                for f in range(f0, f0 + 2 * XP):
                    kb_ref[pr, f, 8 * u:8 * u + 8, :] = bcast(kk, f)

        sub_pc = lax.broadcasted_iota(jnp.int32, (8, PC), 0)

        def qv(c, carry):
            r0 = pl.multiple_of(c * PC, PC)
            xn = xn_ref[pl.ds(r0, PC), :]
            qt = lax.dot_general(wqvt_ref[0:D, :], xn, NT, preferred_element_type=f32)
            qt = (qt * QSCALE).astype(bf16).astype(f32)
            for t in range(PC // 128):
                for g in range(NG):
                    qt_ref[g, c * (PC // 128) + t, 0:GW, :] = qt[g * GW:(g + 1) * GW,
                                                                 t * 128:(t + 1) * 128]
            qn2 = jnp.dot(e2, (qt * qt).astype(bf16), preferred_element_type=f32)
            xv = pltpu.bitcast(
                xv_ref[pl.ds(pl.multiple_of(c * (PC // 2), PC // 2), PC // 2), :], bf16)
            vt = lax.dot_general(wqvt_ref[D:2 * D, :], xv, NT, preferred_element_type=f32)
            negm = M_OFFSET - jnp.sqrt(qn2 * kmax2) * (1.0 + 2.0 ** -6)
            negm = negm.astype(bf16).astype(f32)
            for h in range(H):
                shv = jnp.where((sub_pc == 0) | (sub_pc == 3) | (sub_pc == 4), negm[h:h + 1, :], 0.0)
                for t in range(PC // 128):
                    sh_ref[h, c * (PC // 128) + t, 0:8, :] = shv[:, t * 128:(t + 1) * 128]
                w0 = 8 * ((DH * h) // 8)
                if h % 2 == 0:
                    vw = jnp.concatenate(
                        [vt[w0:w0 + 16], jnp.where(sub_pc < 4, vt[w0 + 16:w0 + 24], 1.0)], axis=0)
                else:
                    vw = jnp.concatenate(
                        [jnp.where(sub_pc >= 4, vt[w0:w0 + 8], 1.0), vt[w0 + 8:w0 + 24]], axis=0)
                vt_ref[h, :, pl.ds(r0, PC)] = vw
            return carry

        lax.fori_loop(0, NPC, qv, 0)

        for cp in late_cp:
            cp.wait()

        def ffn(t, carry):
            r0 = pl.multiple_of(t * TR, TR)
            xn = xn_ref[pl.ds(r0, TR), :]
            y = x_ref[pl.ds(r0, TR), :].astype(f32)
            outs = []
            for c in range(F // FC):
                g = jnp.dot(xn, wg_ref[:, c * FC:(c + 1) * FC], preferred_element_type=f32)
                u = jnp.dot(xn, wu_ref[:, c * FC:(c + 1) * FC], preferred_element_type=f32)
                hh = (g * jax.nn.sigmoid(g) * u).astype(bf16)
                y = y + jnp.dot(hh, wd_ref[c * FC:(c + 1) * FC, :], preferred_element_type=f32)
                outs += [g, u]
            y_ref[pl.ds(r0, TR), :] = y
            if KV:
                nr, ncol = TR // 8, FC // 128
                nv = nr * ncol
                ties = lambda pos: outs[pos // nv][
                    8 * (pos % nr):8 * (pos % nr) + 8,
                    ((pos % nv) // nr) * 128:((pos % nv) // nr + 1) * 128]
                ppi = H // 2 // NR
                make_kb([t * ppi + k for k in range(ppi)], ties, len(outs) * nv)
            return carry

        lax.fori_loop(0, NR, ffn, 0)

        sub = lax.broadcasted_iota(jnp.int32, (8, TQ), 0)

        def load_qm(g, j, t0):
            lo, hi = DH * j, DH * j + DH
            rows = []
            for r in range(GW // 8):
                a, b = 8 * r, 8 * r + 8
                if b <= lo or a >= hi:
                    rows.append(None)
                    continue
                v = jnp.concatenate([qt_ref[g, t0 + t, a:b, :] for t in range(NT128)], axis=1)
                if a < lo:
                    v = jnp.where(sub >= lo - a, v, 0.0)
                elif b > hi:
                    v = jnp.where(sub < hi - a, v, 0.0)
                rows.append(v)
            rows.append(jnp.concatenate(
                [sh_ref[g * HPG + j, t0 + t, 0:8, :] for t in range(NT128)], axis=1))
            rows += [None] * (16 - len(rows))
            blocks = []
            for r in range(8):
                a, b = rows[2 * r], rows[2 * r + 1]
                if a is None and b is None:
                    blocks.append(jnp.zeros((16, TQ), bf16))
                else:
                    a = jnp.zeros((8, TQ), f32) if a is None else a
                    b = jnp.zeros((8, TQ), f32) if b is None else b
                    blocks.append(jnp.concatenate([a, b], axis=0).astype(bf16))
            return jnp.concatenate(blocks, axis=0)

        def vpu_head(it, i, tok):
            ib = it // NQ
            t0 = (it % NQ) * NT128
            g, j = ib * GPI + i // HPG, i % HPG
            h = g * HPG + j
            for t in range(NT128):
                for a in range(0, KV, 16):
                    qrow = lambda d: qt_ref[g, t0 + t, pl.ds(j * DH + d, 8, stride=0), :]
                    srow = lambda r: sh_ref[h, t0 + t, pl.ds(r, 8, stride=0), :]
                    if tok is None or tok is False:
                        init = srow(3)
                    else:
                        init = jnp.where(tok > 0.0, srow(3), srow(4))
                    acc = [init, init]
                    for d in range(DH):
                        qb = qrow(d)
                        for u in range(2):
                            kb = kb_ref[ib * (NH // 2) + i // 2, (i % 2) * DH + d,
                                        a + 8 * u:a + 8 * u + 8, :]
                            acc[u] = acc[u] + kb * qb
                    pk = interleave_pack(jnp.exp2(jnp.concatenate(acc, axis=0)))
                    r0 = (KL - KV + a) // 2
                    pl_ref[i, r0:r0 + 8, t * 128:(t + 1) * 128] = pk
                    if tok is not False:
                        tok = pltpu.bitcast(pk, f32)
            return tok

        def attn_step(it, bad):
            ib = it // NQ
            g0 = ib * GPI
            t0 = (it % NQ) * NT128
            q0 = pl.multiple_of((it % NQ) * TQ, TQ)
            qms = [None] * NH
            accs = [None] * NH
            nc = len(mchunks)
            steps = [(i, c) for i in range(NH) for c in range(nc)]
            tok = [None]
            zz = z_ref[0] if PDYN else 0

            def qk(n):
                i, c = steps[n]
                a, b = mchunks[c]
                g = g0 + i // HPG
                if qms[i] is None:
                    qms[i] = load_qm(g, i % HPG, t0)
                    if KV and i + 1 < NH:
                        tok[0] = vpu_head(it, i + 1, tok[0])
                    elif KV:
                        tok[0] = vpu_head((it + 1) % (NI * NQ), 0, tok[0])
                st = jnp.dot(k_ref[g, a:b, :], qms[i], preferred_element_type=f32)
                if b == KM and KL > KV and i > 0:
                    pl_ref[i, 0:(b - a) // 2, :] = interleave_pack(jnp.exp2(st))
                else:
                    pbuf[n % NPB][zz, 0:(b - a) // 2, :] = interleave_pack(jnp.exp2(st))

            def finish(i, bad):
                outs = []
                for odd, a in enumerate((accs[i], accs[i + 1])):
                    lv = a[0:8] if odd else a[16:24]
                    keep = (sub < 4) if odd else (sub >= 4)
                    l = jnp.where(keep, lv, pltpu.roll(lv, 4, 0))
                    r = 1.0 / l
                    amax = jnp.maximum(jnp.maximum(jnp.abs(a[0:8]), jnp.abs(a[8:16])),
                                       jnp.abs(a[16:24]))
                    ok = (l >= L_MIN) & (amax <= ACC_MAX)
                    bad = jnp.where(ok, bad, 1.0)
                    outs.append([a[0:8] * r, a[8:16] * r, a[16:24] * r])
                mid = jnp.where(sub < 4, outs[0][2], outs[1][0])
                o = jnp.concatenate([outs[0][0], outs[0][1], mid, outs[1][1], outs[1][2]], axis=0)
                ot_ref[pl.ds(pl.multiple_of(g0 * GW + i * DH, 8), 40), pl.ds(q0, TQ)] = o
                return bad

            def pv(i, a, b, pu):
                r = lax.dot_general(vt_ref[g0 * HPG + i, :, a:b], pltpu.bitcast(pu, bf16), NN,
                                    preferred_element_type=f32)
                accs[i] = r if accs[i] is None else accs[i] + r

            pv0 = pl_ref[0, (KL - KV) // 2:, :] if KV else None
            for n in range(DEPTH):
                qk(n)
            for n, (i, c) in enumerate(steps):
                a, b = mchunks[c]
                if n + DEPTH < len(steps):
                    qk(n + DEPTH)
                if not (b == KM and KL > KV and i > 0):
                    pv(i, a, b, pbuf[n % NPB][zz, 0:(b - a) // 2, :])
                if KV and i == 0 and c == 0:
                    pv(i, KM, S, pv0)
                if KV and i > 0 and c == nc - 1:
                    pv(i, S - KL, S, pl_ref[i])
                if i % 2 == 1 and c == nc - 1:
                    bad = finish(i - 1, bad)
            return bad

        def true_max():
            rows80 = lax.broadcasted_iota(jnp.int32, (GW, TQ), 0)

            def one(it, carry):
                h = it // NQ
                t0 = (it % NQ) * NT128
                g = h // HPG
                lo = (h % HPG) * DH
                win = jnp.concatenate([qt_ref[g, t0 + t, 0:GW, :] for t in range(NT128)], axis=1)
                qm = jnp.concatenate(
                    [jnp.where((rows80 >= lo) & (rows80 < lo + DH), win, 0.0),
                     jnp.zeros((128 - GW, TQ), f32)], axis=0).astype(bf16)

                def chunk(c, mx):
                    st = jnp.dot(k_ref[g, pl.ds(pl.multiple_of(c * 256, 256), 256), :], qm,
                                 preferred_element_type=f32)
                    return jnp.maximum(mx, jnp.max(st, axis=0, keepdims=True))

                mx = lax.fori_loop(0, S // 256, chunk, jnp.full((1, TQ), -jnp.inf, f32))
                m1 = mx.astype(bf16).astype(f32)
                m2 = (mx - m1).astype(bf16).astype(f32)
                m3 = (mx - m1 - m2).astype(bf16).astype(f32)
                shv = jnp.where(sub == 0, -m1, jnp.where(sub == 1, -m2, jnp.where(
                    sub == 2, -m3, jnp.where((sub == 3) | (sub == 4), -(m1 + m2 + m3), 0.0))))
                for t in range(NT128):
                    sh_ref[h, t0 + t, 0:8, :] = shv[:, t * 128:(t + 1) * 128]
                return carry

            lax.fori_loop(0, H * NQ, one, 0)

        NSTEP = NI * NQ if N1 is None else N1

        def attempt(state):
            n, _ = state

            @pl.when(n > 0)
            def _():
                true_max()

            if KV:
                vpu_head(0, 0, False)
            bad = lax.fori_loop(0, NSTEP, attn_step, jnp.zeros((8, TQ), f32))
            unsafe = jnp.max(bad) > (-1.0 if FORCE_FALLBACK else (5.0 if NOCHECK else 0.0))
            return n + 1, unsafe.astype(jnp.int32)

        lax.while_loop(lambda s: (s[0] < 2) & (s[1] > 0), attempt,
                       (jnp.int32(0), jnp.int32(1)))

        out_cp = [pltpu.make_async_copy(ob_ref.at[t * TO:(t + 1) * TO],
                                        o_hbm.at[t * TO:(t + 1) * TO], sem_o.at[t])
                  for t in range(S // TO)]
        for t in range(S // TO):
            a, b = t * TO, (t + 1) * TO
            y = y_ref[a:b, :] + lax.dot_general(ot_ref[:, a:b].astype(bf16), wo_ref[...], TN,
                                                preferred_element_type=f32)
            ob_ref[a:b, :] = y.astype(bf16)
            out_cp[t].start()
        for cp in out_cp:
            cp.wait()

    def run(A_x, A_wqkv, A_wo, B_x, B_w_gate, B_w_up, B_w_down):
        x = A_x.reshape(S, D)
        anyspec = pl.BlockSpec(memory_space=pl.ANY)
        kvs = max(KV, 8)
        out = pl.pallas_call(
            kernel,
            in_specs=[anyspec] * 6,
            out_specs=anyspec,
            out_shape=jax.ShapeDtypeStruct((S, D), bf16),
            scratch_shapes=[
                pltpu.VMEM((S, D), bf16),
                pltpu.VMEM((D, 3 * D), bf16),
                pltpu.VMEM((D, D), bf16),
                pltpu.VMEM((D, F), bf16),
                pltpu.VMEM((D, F), bf16),
                pltpu.VMEM((F, D), bf16),
                pltpu.VMEM((S, D), bf16),
                pltpu.VMEM((S, D), bf16),
                pltpu.VMEM((S // 2, D), u32),
                pltpu.VMEM((NG, S, 128), bf16),
                pltpu.VMEM((NG, S // 128, GW + 8, 128), f32),
                pltpu.VMEM((H, S // 128, 16, 128), f32),
                pltpu.VMEM((H, 24, S), f32),
                pltpu.VMEM((2 * D, D), bf16),
                pltpu.VMEM((H, S), f32),
                pltpu.VMEM((D, S), f32),
                pltpu.VMEM((NH, max(KL, 16) // 2, TQ), u32),
                pltpu.VMEM((2, H // 2, kvs, 128), f32),
                pltpu.VMEM((H // 2, 2 * DH, kvs, 128), f32),
                pltpu.VMEM((S, D), f32),
                pltpu.SemaphoreType.DMA((NK,)),
                pltpu.SemaphoreType.DMA((7,)),
                pltpu.SemaphoreType.DMA((S // TO,)),
                pltpu.SMEM((1,), jnp.int32),
            ] + [pltpu.VMEM((2, KC // 2, TQ), u32) for _ in range(NPB)],
            compiler_params=pltpu.CompilerParams(vmem_limit_bytes=126 * 1024 * 1024),
        )(x, A_wqkv, A_wo, B_w_gate, B_w_up, B_w_down)
        return out.reshape(1, S, D)

    return run


_run = make_kernel(KV=160)


@jax.jit
def pallas_parallel_sum__mha_block__swiglu_ffn__prompt_kernel(
    A_x: jax.Array,
    A_wqkv: jax.Array,
    A_wo: jax.Array,
    B_x: jax.Array,
    B_w_gate: jax.Array,
    B_w_up: jax.Array,
    B_w_down: jax.Array,
):
    return _run(A_x, A_wqkv, A_wo, B_x, B_w_gate, B_w_up, B_w_down)
```

```python
import math

import jax
import jax.numpy as jnp
from jax import lax
import jax.experimental.pallas as pl
import jax.experimental.pallas.tpu as pltpu

S, D, H, DH, F = 2048, 640, 32, 20, 1536
HPG = 4
NG = H // HPG
GW = HPG * DH
GPI = 2
NH = GPI * HPG
NI = NG // GPI
QSCALE = (DH ** -0.5) * math.log2(math.e)
M_OFFSET = 72.0
L_MIN = 2.0 ** -40
ACC_MAX = 2.0 ** 120

f32 = jnp.float32
bf16 = jnp.bfloat16
u32 = jnp.uint32
NT = (((1,), (1,)), ((), ()))
TN = (((0,), (0,)), ((), ()))
NN = (((1,), (0,)), ((), ()))

TQ = 512
NT128 = TQ // 128
NQ = S // TQ
PC = 512
NPC = S // PC


def make_kernel(KC=128, DEPTH=5, TR=256, FC=512, NPB=8, MS=128, KV=160, XP=10, TO=256,
                FORCE_FALLBACK=False, INTERP=False):
    NR = S // TR
    KM = S - KV
    KL = -(-KV // 128) * 128
    KR = KL - KV
    mchunks = [(c, min(c + KC, S - KL)) for c in range(0, S - KL, KC)]
    if KR:
        mchunks.append((S - KL, KM))
    assert KV % 16 == 0 and KV > 0 and (2 * DH) % XP == 0 and (H // 2) % NR == 0

    def pair_pack(v, rnd=False):
        n, m = v.shape
        u = lax.bitcast_convert_type(v, u32)
        if rnd:
            u = u + jnp.uint32(0x8000)
        e = u.reshape(n // 16, 2, 8, m)
        lo = lax.shift_right_logical(e[:, 0].reshape(n // 2, m), jnp.uint32(16))
        hi = e[:, 1].reshape(n // 2, m) & jnp.uint32(0xFFFF0000)
        return lo | hi

    def kernel(x_hbm, wqkv_hbm, wo_hbm, wg_hbm, wu_hbm, wd_hbm, o_hbm,
               x_ref, wqkv_ref, wo_ref, wg_ref, wu_ref, wd_ref, ob_ref,
               xn_ref, xv_ref, k_ref, qt_ref, sh_ref, vt_ref, wqvt_ref, kn2_ref, ot_ref,
               pl_ref, kf_ref, kb_ref, y_ref, sem_x, sem_w, sem_o, z_ref, *pbuf):
        z_ref[0] = 0
        x_cp = [pltpu.make_async_copy(x_hbm.at[c * PC:(c + 1) * PC], x_ref.at[c * PC:(c + 1) * PC],
                                      sem_x.at[c]) for c in range(NPC)]
        wk_cp, wq_cp, wv_cp = [
            pltpu.make_async_copy(wqkv_hbm.at[:, a:a + D], wqkv_ref.at[:, a:a + D], sem_w.at[i])
            for i, a in enumerate((D, 0, 2 * D))]
        late_cp = [pltpu.make_async_copy(s, d, sem_w.at[3 + i]) for i, (s, d) in enumerate(
            [(wg_hbm, wg_ref), (wu_hbm, wu_ref), (wd_hbm, wd_ref), (wo_hbm, wo_ref)])]
        x_cp[0].start()
        wk_cp.start()
        for c in range(1, NPC):
            x_cp[c].start()
        wq_cp.start()
        wv_cp.start()

        def layernorm(c):
            a, b = c * PC, (c + 1) * PC
            x = x_ref[a:b, :].astype(f32)
            mu = jnp.mean(x, axis=-1, keepdims=True)
            xc = x - mu
            var = jnp.mean(xc * xc, axis=-1, keepdims=True)
            xnf = xc * lax.rsqrt(var + 1e-5)
            xn_ref[a:b, :] = xnf.astype(bf16)
            xv_ref[a // 2:b // 2, :] = pair_pack(xnf, True)

        er2 = lax.broadcasted_iota(jnp.int32, (H, D), 0)
        ec2 = lax.broadcasted_iota(jnp.int32, (H, D), 1)
        e2 = jnp.where((ec2 >= er2 * DH) & (ec2 < er2 * DH + DH), 1.0, 0.0).astype(bf16)
        kconst = jnp.where(lax.broadcasted_iota(jnp.int32, (PC, 128 - GW), 1) < 3, 1.0, 0.0)

        def kproj(c):
            a, b = c * PC, (c + 1) * PC
            kall = jnp.concatenate([
                jnp.dot(xn_ref[m:m + MS, :], wqkv_ref[:, D:2 * D], preferred_element_type=f32)
                for m in range(a, b, MS)], axis=0)
            kn2_ref[:, a:b] = lax.dot_general(e2, (kall * kall).astype(bf16), NT,
                                              preferred_element_type=f32)
            for g in range(NG):
                k_ref[g, a:b, :] = jnp.concatenate(
                    [kall[:, g * GW:(g + 1) * GW], kconst], axis=1).astype(bf16)
            if b == S:
                kv = kall[PC - KV:, :].astype(bf16).astype(f32)
                for pr in range(H // 2):
                    blk = jnp.concatenate([kv[:, 2 * DH * pr:2 * DH * (pr + 1)],
                                           jnp.zeros((KV, 128 - 2 * DH), f32)], axis=1)
                    kf_ref[0, pr] = blk
                    kf_ref[1, pr] = blk

        x_cp[0].wait()
        layernorm(0)
        wk_cp.wait()
        x_cp[1].wait()
        kproj(0)
        layernorm(1)
        for c in range(2, NPC):
            x_cp[c].wait()
        for c in range(1, NPC - 1):
            kproj(c)
            layernorm(c + 1)
        wq_cp.wait()
        wv_cp.wait()
        for cp in late_cp:
            cp.start()
        kproj(NPC - 1)
        wqvt_ref[0:D, :] = wqkv_ref[:, 0:D].astype(f32).T.astype(bf16)
        wqvt_ref[D:2 * D, :] = wqkv_ref[:, 2 * D:3 * D].astype(f32).T.astype(bf16)

        kmax2 = jnp.max(kn2_ref[...], axis=-1, keepdims=True)

        sub_pc = lax.broadcasted_iota(jnp.int32, (8, PC), 0)

        def qv(c, carry):
            r0 = pl.multiple_of(c * PC, PC)
            xn = xn_ref[pl.ds(r0, PC), :]
            qt = lax.dot_general(wqvt_ref[0:D, :], xn, NT, preferred_element_type=f32)
            qt = (qt * QSCALE).astype(bf16).astype(f32)
            for t in range(PC // 128):
                for g in range(NG):
                    qt_ref[g, c * (PC // 128) + t] = qt[g * GW:(g + 1) * GW, t * 128:(t + 1) * 128]
            qn2 = jnp.dot(e2, (qt * qt).astype(bf16), preferred_element_type=f32)
            xv = pltpu.bitcast(
                xv_ref[pl.ds(pl.multiple_of(c * (PC // 2), PC // 2), PC // 2), :], bf16)
            vt = lax.dot_general(wqvt_ref[D:2 * D, :], xv, NT, preferred_element_type=f32)
            negm = M_OFFSET - jnp.sqrt(qn2 * kmax2) * (1.0 + 2.0 ** -6)
            negm = negm.astype(bf16).astype(f32)
            for h in range(H):
                shv = jnp.where((sub_pc == 0) | (sub_pc == 3) | (sub_pc == 4), negm[h:h + 1, :], 0.0)
                for t in range(PC // 128):
                    sh_ref[h, c * (PC // 128) + t] = shv[:, t * 128:(t + 1) * 128]
                w0 = 8 * ((DH * h) // 8)
                if h % 2 == 0:
                    vw = jnp.concatenate(
                        [vt[w0:w0 + 16], jnp.where(sub_pc < 4, vt[w0 + 16:w0 + 24], 1.0)], axis=0)
                else:
                    vw = jnp.concatenate(
                        [jnp.where(sub_pc >= 4, vt[w0:w0 + 8], 1.0), vt[w0 + 8:w0 + 24]], axis=0)
                vt_ref[h, :, pl.ds(r0, PC)] = vw
            return carry

        lax.fori_loop(0, NPC, qv, 0)

        for cp in late_cp:
            cp.wait()

        def ffn(t, carry):
            r0 = pl.multiple_of(t * TR, TR)
            xn = xn_ref[pl.ds(r0, TR), :]
            y = x_ref[pl.ds(r0, TR), :].astype(f32)
            outs = []
            for c in range(F // FC):
                g = jnp.dot(xn, wg_ref[:, c * FC:(c + 1) * FC], preferred_element_type=f32)
                u = jnp.dot(xn, wu_ref[:, c * FC:(c + 1) * FC], preferred_element_type=f32)
                hh = (g * jax.nn.sigmoid(g) * u).astype(bf16)
                y = y + jnp.dot(hh, wd_ref[c * FC:(c + 1) * FC, :], preferred_element_type=f32)
                outs += [g, u]
            y_ref[pl.ds(r0, TR), :] = y
            nr = TR // 8
            nv = nr * (FC // 128)
            ppi = H // 2 // NR
            jobs = [(k, u, f0) for k in range(ppi) for u in range(KV // 8)
                    for f0 in range(0, 2 * DH, XP)]
            for n, (k, u, f0) in enumerate(jobs):
                pos = n * len(outs) * nv // len(jobs)
                r, col = pos % nr, (pos % nv) // nr
                tie = outs[pos // nv][8 * r:8 * r + 8, col * 128:(col + 1) * 128]
                pr = t * ppi + k
                kk = jnp.where(tie > 0.0, kf_ref[0, pr, 8 * u:8 * u + 8, :],
                               kf_ref[1, pr, 8 * u:8 * u + 8, :])
                for f in range(f0, f0 + XP):
                    kb_ref[pr, f, 8 * u:8 * u + 8, :] = jnp.broadcast_to(kk[:, f:f + 1], (8, 128))
            return carry

        lax.fori_loop(0, NR, ffn, 0)

        sub = lax.broadcasted_iota(jnp.int32, (8, TQ), 0)

        def load_qm(g, j, t0):
            lo, hi = DH * j, DH * j + DH
            rows = []
            for r in range(GW // 8):
                a, b = 8 * r, 8 * r + 8
                if b <= lo or a >= hi:
                    rows.append(None)
                    continue
                v = jnp.concatenate([qt_ref[g, t0 + t, a:b, :] for t in range(NT128)], axis=1)
                if a < lo:
                    v = jnp.where(sub >= lo - a, v, 0.0)
                elif b > hi:
                    v = jnp.where(sub < hi - a, v, 0.0)
                rows.append(v)
            rows.append(jnp.concatenate(
                [sh_ref[g * HPG + j, t0 + t] for t in range(NT128)], axis=1))
            rows += [None] * (16 - len(rows))
            blocks = []
            for r in range(8):
                a, b = rows[2 * r], rows[2 * r + 1]
                if a is None and b is None:
                    blocks.append(jnp.zeros((16, TQ), bf16))
                else:
                    a = jnp.zeros((8, TQ), f32) if a is None else a
                    b = jnp.zeros((8, TQ), f32) if b is None else b
                    blocks.append(jnp.concatenate([a, b], axis=0).astype(bf16))
            return jnp.concatenate(blocks, axis=0)

        def vpu_head(it, i, tok):
            ib = it // NQ
            t0 = (it % NQ) * NT128
            g, j = ib * GPI + i // HPG, i % HPG
            for t in range(NT128):
                qrow = [jnp.broadcast_to(qt_ref[g, t0 + t, j * DH + d:j * DH + d + 1, :], (8, 128))
                        for d in range(DH)]
                srow = [jnp.broadcast_to(sh_ref[g * HPG + j, t0 + t, r:r + 1, :], (8, 128))
                        for r in (3, 4)]
                for a in range(0, KV, 16):
                    init = srow[0] if tok is None else jnp.where(tok > 0.0, srow[0], srow[1])
                    acc = [init, init]
                    for d in range(DH):
                        for u in range(2):
                            acc[u] = acc[u] + qrow[d] * kb_ref[
                                ib * (NH // 2) + i // 2, (i % 2) * DH + d,
                                a + 8 * u:a + 8 * u + 8, :]
                    pk = pair_pack(jnp.exp2(jnp.concatenate(acc, axis=0)))
                    r0 = (KR + a) // 2
                    pl_ref[i, r0:r0 + 8, t * 128:(t + 1) * 128] = pk
                    tok = lax.bitcast_convert_type(pk, f32)
            return tok

        def attn_step(it, bad):
            g0 = (it // NQ) * GPI
            t0 = (it % NQ) * NT128
            q0 = pl.multiple_of((it % NQ) * TQ, TQ)
            qms = [None] * NH
            accs = [None] * NH
            nc = len(mchunks)
            steps = [(i, c) for i in range(NH) for c in range(nc)]
            tok = [None]
            zz = z_ref[0]

            def in_last_block(i, b):
                return b == KM and KR > 0 and i > 0

            def qk(n):
                i, c = steps[n]
                a, b = mchunks[c]
                g = g0 + i // HPG
                if qms[i] is None:
                    qms[i] = load_qm(g, i % HPG, t0)
                    if i + 1 < NH:
                        tok[0] = vpu_head(it, i + 1, tok[0])
                    else:
                        tok[0] = vpu_head((it + 1) % (NI * NQ), 0, tok[0])
                st = jnp.dot(k_ref[g, a:b, :], qms[i], preferred_element_type=f32)
                if in_last_block(i, b):
                    pl_ref[i, 0:(b - a) // 2, :] = pair_pack(jnp.exp2(st))
                else:
                    pbuf[n % NPB][zz, 0:(b - a) // 2, :] = pair_pack(jnp.exp2(st))

            def pv(i, a, b, pu):
                r = lax.dot_general(vt_ref[g0 * HPG + i, :, a:b], pltpu.bitcast(pu, bf16), NN,
                                    preferred_element_type=f32)
                accs[i] = r if accs[i] is None else accs[i] + r

            def finish(i, bad):
                outs = []
                for odd, a in enumerate((accs[i], accs[i + 1])):
                    lv = a[0:8] if odd else a[16:24]
                    keep = (sub < 4) if odd else (sub >= 4)
                    l = jnp.where(keep, lv, pltpu.roll(lv, 4, 0))
                    r = 1.0 / l
                    amax = jnp.maximum(jnp.maximum(jnp.abs(a[0:8]), jnp.abs(a[8:16])),
                                       jnp.abs(a[16:24]))
                    ok = (l >= L_MIN) & (amax <= ACC_MAX)
                    bad = jnp.where(ok, bad, 1.0)
                    outs.append([a[0:8] * r, a[8:16] * r, a[16:24] * r])
                mid = jnp.where(sub < 4, outs[0][2], outs[1][0])
                o = jnp.concatenate([outs[0][0], outs[0][1], mid, outs[1][1], outs[1][2]], axis=0)
                ot_ref[pl.ds(pl.multiple_of(g0 * GW + i * DH, 8), 40), pl.ds(q0, TQ)] = o
                return bad

            pv0 = pl_ref[0, KR // 2:, :]
            for n in range(DEPTH):
                qk(n)
            for n, (i, c) in enumerate(steps):
                a, b = mchunks[c]
                if n + DEPTH < len(steps):
                    qk(n + DEPTH)
                if not in_last_block(i, b):
                    pv(i, a, b, pbuf[n % NPB][zz, 0:(b - a) // 2, :])
                if i == 0 and c == 0:
                    pv(i, KM, S, pv0)
                if i > 0 and c == nc - 1:
                    pv(i, S - KL, S, pl_ref[i])
                if i % 2 == 1 and c == nc - 1:
                    bad = finish(i - 1, bad)
            return bad

        def true_max():
            rows80 = lax.broadcasted_iota(jnp.int32, (GW, TQ), 0)

            def one(it, carry):
                h = it // NQ
                t0 = (it % NQ) * NT128
                g = h // HPG
                lo = (h % HPG) * DH
                win = jnp.concatenate([qt_ref[g, t0 + t] for t in range(NT128)], axis=1)
                qm = jnp.concatenate(
                    [jnp.where((rows80 >= lo) & (rows80 < lo + DH), win, 0.0),
                     jnp.zeros((128 - GW, TQ), f32)], axis=0).astype(bf16)

                def chunk(c, mx):
                    st = jnp.dot(k_ref[g, pl.ds(pl.multiple_of(c * 256, 256), 256), :], qm,
                                 preferred_element_type=f32)
                    return jnp.maximum(mx, jnp.max(st, axis=0, keepdims=True))

                mx = lax.fori_loop(0, S // 256, chunk, jnp.full((1, TQ), -jnp.inf, f32))
                m1 = mx.astype(bf16).astype(f32)
                m2 = (mx - m1).astype(bf16).astype(f32)
                m3 = (mx - m1 - m2).astype(bf16).astype(f32)
                shv = jnp.where(sub == 0, -m1, jnp.where(sub == 1, -m2, jnp.where(
                    sub == 2, -m3, jnp.where((sub == 3) | (sub == 4), -(m1 + m2 + m3), 0.0))))
                for t in range(NT128):
                    sh_ref[h, t0 + t] = shv[:, t * 128:(t + 1) * 128]
                return carry

            lax.fori_loop(0, H * NQ, one, 0)

        def attempt(state):
            n, _ = state

            @pl.when(n > 0)
            def _():
                true_max()

            pl_ref[0, KR // 2:, :] = pair_pack(jnp.exp2(jnp.dot(
                k_ref[0, KM:S, :], load_qm(0, 0, 0), preferred_element_type=f32)))
            bad = lax.fori_loop(0, NI * NQ, attn_step, jnp.zeros((8, TQ), f32))
            unsafe = jnp.max(bad) > (-1.0 if FORCE_FALLBACK else 0.0)
            return n + 1, unsafe.astype(jnp.int32)

        lax.while_loop(lambda s: (s[0] < 2) & (s[1] > 0), attempt,
                       (jnp.int32(0), jnp.int32(1)))

        out_cp = [pltpu.make_async_copy(ob_ref.at[t * TO:(t + 1) * TO],
                                        o_hbm.at[t * TO:(t + 1) * TO], sem_o.at[t])
                  for t in range(S // TO)]
        for t in range(S // TO):
            a, b = t * TO, (t + 1) * TO
            y = y_ref[a:b, :] + lax.dot_general(ot_ref[:, a:b].astype(bf16), wo_ref[...], TN,
                                                preferred_element_type=f32)
            ob_ref[a:b, :] = y.astype(bf16)
            out_cp[t].start()
        for cp in out_cp:
            cp.wait()

    def run(A_x, A_wqkv, A_wo, B_x, B_w_gate, B_w_up, B_w_down):
        x = A_x.reshape(S, D)
        anyspec = pl.BlockSpec(memory_space=pl.ANY)
        out = pl.pallas_call(
            kernel,
            in_specs=[anyspec] * 6,
            out_specs=anyspec,
            out_shape=jax.ShapeDtypeStruct((S, D), bf16),
            scratch_shapes=[
                pltpu.VMEM((S, D), bf16),
                pltpu.VMEM((D, 3 * D), bf16),
                pltpu.VMEM((D, D), bf16),
                pltpu.VMEM((D, F), bf16),
                pltpu.VMEM((D, F), bf16),
                pltpu.VMEM((F, D), bf16),
                pltpu.VMEM((S, D), bf16),
                pltpu.VMEM((S, D), bf16),
                pltpu.VMEM((S // 2, D), u32),
                pltpu.VMEM((NG, S, 128), bf16),
                pltpu.VMEM((NG, S // 128, GW, 128), f32),
                pltpu.VMEM((H, S // 128, 8, 128), f32),
                pltpu.VMEM((H, 24, S), f32),
                pltpu.VMEM((2 * D, D), bf16),
                pltpu.VMEM((H, S), f32),
                pltpu.VMEM((D, S), f32),
                pltpu.VMEM((NH, KL // 2, TQ), u32),
                pltpu.VMEM((2, H // 2, KV, 128), f32),
                pltpu.VMEM((H // 2, 2 * DH, KV, 128), f32),
                pltpu.VMEM((S, D), f32),
                pltpu.SemaphoreType.DMA((NPC,)),
                pltpu.SemaphoreType.DMA((7,)),
                pltpu.SemaphoreType.DMA((S // TO,)),
                pltpu.SMEM((1,), jnp.int32),
            ] + [pltpu.VMEM((2, KC // 2, TQ), u32) for _ in range(NPB)],
            compiler_params=pltpu.CompilerParams(vmem_limit_bytes=126 * 1024 * 1024),
            interpret=INTERP,
        )(x, A_wqkv, A_wo, B_w_gate, B_w_up, B_w_down)
        return out.reshape(1, S, D)

    return run


_run = make_kernel(TO=128)


@jax.jit
def pallas_parallel_sum__mha_block__swiglu_ffn__prompt_kernel(
    A_x: jax.Array,
    A_wqkv: jax.Array,
    A_wo: jax.Array,
    B_x: jax.Array,
    B_w_gate: jax.Array,
    B_w_up: jax.Array,
    B_w_down: jax.Array,
):
    return _run(A_x, A_wqkv, A_wo, B_x, B_w_gate, B_w_up, B_w_down)
```

```python
import math

import jax
import jax.numpy as jnp
from jax import lax
import jax.experimental.pallas as pl
import jax.experimental.pallas.tpu as pltpu

S, D, H, DH, F = 2048, 640, 32, 20, 1536
HPG = 4
NG = H // HPG
GW = HPG * DH
GPI = 2
NH = GPI * HPG
NI = NG // GPI
QSCALE = (DH ** -0.5) * math.log2(math.e)
M_OFFSET = 72.0
L_MIN = 2.0 ** -40
ACC_MAX = 2.0 ** 120

f32 = jnp.float32
bf16 = jnp.bfloat16
u32 = jnp.uint32
NT = (((1,), (1,)), ((), ()))
TN = (((0,), (0,)), ((), ()))
NN = (((1,), (0,)), ((), ()))

TQ = 512
NT128 = TQ // 128
NQ = S // TQ
PC = 512
NPC = S // PC


def make_kernel(KC=128, DEPTH=5, TR=256, FC=512, NPB=8, MS=64, KV=160, XP=10, TO=128,
                FORCE_FALLBACK=False, INTERP=False, BL=(512, 1536), SUB=512):
    NR = S // TR
    blocks = list(zip((0,) + tuple(BL), tuple(BL) + (S,)))
    KM = S - KV
    KL = -(-KV // 128) * 128
    KR = KL - KV
    mchunks = [(c, min(c + KC, S - KL)) for c in range(0, S - KL, KC)]
    if KR:
        mchunks.append((S - KL, KM))
    assert KV % 16 == 0 and KV > 0 and (2 * DH) % XP == 0 and (H // 2) % NR == 0

    def pair_pack(v, rnd=False):
        n, m = v.shape
        u = lax.bitcast_convert_type(v, u32)
        if rnd:
            u = u + jnp.uint32(0x8000)
        e = u.reshape(n // 16, 2, 8, m)
        lo = lax.shift_right_logical(e[:, 0].reshape(n // 2, m), jnp.uint32(16))
        hi = e[:, 1].reshape(n // 2, m) & jnp.uint32(0xFFFF0000)
        return lo | hi

    def kernel(x_hbm, wqkv_hbm, wo_hbm, wg_hbm, wu_hbm, wd_hbm, o_hbm,
               x_ref, wqkv_ref, wo_ref, wg_ref, wu_ref, wd_ref, ob_ref,
               xn_ref, xv_ref, k_ref, qt_ref, sh_ref, vt_ref, wqvt_ref, kn2_ref, ot_ref,
               pl_ref, kf_ref, kb_ref, y_ref, sem_x, sem_w, sem_o, z_ref, *pbuf):
        z_ref[0] = 0
        x_cp = [pltpu.make_async_copy(x_hbm.at[a:b], x_ref.at[a:b], sem_x.at[c])
                for c, (a, b) in enumerate(blocks)]
        wk_cp, wq_cp, wv_cp = [
            pltpu.make_async_copy(wqkv_hbm.at[:, a:a + D], wqkv_ref.at[:, a:a + D], sem_w.at[i])
            for i, a in enumerate((D, 0, 2 * D))]
        late_cp = [pltpu.make_async_copy(s, d, sem_w.at[3 + i]) for i, (s, d) in enumerate(
            [(wg_hbm, wg_ref), (wu_hbm, wu_ref), (wd_hbm, wd_ref), (wo_hbm, wo_ref)])]
        x_cp[0].start()
        wk_cp.start()
        for cp in x_cp[1:]:
            cp.start()
        wq_cp.start()
        wv_cp.start()

        def layernorm(a, b):
            x = x_ref[a:b, :].astype(f32)
            mu = jnp.mean(x, axis=-1, keepdims=True)
            xc = x - mu
            var = jnp.mean(xc * xc, axis=-1, keepdims=True)
            xnf = xc * lax.rsqrt(var + 1e-5)
            xn_ref[a:b, :] = xnf.astype(bf16)
            xv_ref[a // 2:b // 2, :] = pair_pack(xnf, True)

        er2 = lax.broadcasted_iota(jnp.int32, (H, D), 0)
        ec2 = lax.broadcasted_iota(jnp.int32, (H, D), 1)
        e2 = jnp.where((ec2 >= er2 * DH) & (ec2 < er2 * DH + DH), 1.0, 0.0).astype(bf16)
        def kproj(a, b):
            kconst = jnp.where(lax.broadcasted_iota(jnp.int32, (b - a, 128 - GW), 1) < 3, 1.0, 0.0)
            kall = jnp.concatenate([
                jnp.dot(xn_ref[m:m + MS, :], wqkv_ref[:, D:2 * D], preferred_element_type=f32)
                for m in range(a, b, MS)], axis=0)
            kn2_ref[:, a:b] = lax.dot_general(e2, (kall * kall).astype(bf16), NT,
                                              preferred_element_type=f32)
            for g in range(NG):
                k_ref[g, a:b, :] = jnp.concatenate(
                    [kall[:, g * GW:(g + 1) * GW], kconst], axis=1).astype(bf16)
            if b == S:
                kv = kall[b - a - KV:, :].astype(bf16).astype(f32)
                for pr in range(H // 2):
                    blk = jnp.concatenate([kv[:, 2 * DH * pr:2 * DH * (pr + 1)],
                                           jnp.zeros((KV, 128 - 2 * DH), f32)], axis=1)
                    kf_ref[0, pr] = blk
                    kf_ref[1, pr] = blk

        for c, (a, b) in enumerate(blocks):
            x_cp[c].wait()
            if c == 0:
                layernorm(a, b)
                wk_cp.wait()
                kproj(a, b)
                continue
            if c == len(blocks) - 1:
                wq_cp.wait()
                wv_cp.wait()
                for cp in late_cp:
                    cp.start()
            for m in range(a, b, SUB):
                layernorm(m, min(m + SUB, b))
                kproj(m, min(m + SUB, b))
        wqvt_ref[0:D, :] = wqkv_ref[:, 0:D].astype(f32).T.astype(bf16)
        wqvt_ref[D:2 * D, :] = wqkv_ref[:, 2 * D:3 * D].astype(f32).T.astype(bf16)

        kmax2 = jnp.max(kn2_ref[...], axis=-1, keepdims=True)

        sub_pc = lax.broadcasted_iota(jnp.int32, (8, PC), 0)

        def qv(c, carry):
            r0 = pl.multiple_of(c * PC, PC)
            xn = xn_ref[pl.ds(r0, PC), :]
            qt = lax.dot_general(wqvt_ref[0:D, :], xn, NT, preferred_element_type=f32)
            qt = (qt * QSCALE).astype(bf16).astype(f32)
            for t in range(PC // 128):
                for g in range(NG):
                    qt_ref[g, c * (PC // 128) + t] = qt[g * GW:(g + 1) * GW, t * 128:(t + 1) * 128]
            qn2 = jnp.dot(e2, (qt * qt).astype(bf16), preferred_element_type=f32)
            xv = pltpu.bitcast(
                xv_ref[pl.ds(pl.multiple_of(c * (PC // 2), PC // 2), PC // 2), :], bf16)
            vt = lax.dot_general(wqvt_ref[D:2 * D, :], xv, NT, preferred_element_type=f32)
            negm = M_OFFSET - jnp.sqrt(qn2 * kmax2) * (1.0 + 2.0 ** -6)
            negm = negm.astype(bf16).astype(f32)
            for h in range(H):
                shv = jnp.where((sub_pc == 0) | (sub_pc == 3) | (sub_pc == 4), negm[h:h + 1, :], 0.0)
                for t in range(PC // 128):
                    sh_ref[h, c * (PC // 128) + t] = shv[:, t * 128:(t + 1) * 128]
                w0 = 8 * ((DH * h) // 8)
                if h % 2 == 0:
                    vw = jnp.concatenate(
                        [vt[w0:w0 + 16], jnp.where(sub_pc < 4, vt[w0 + 16:w0 + 24], 1.0)], axis=0)
                else:
                    vw = jnp.concatenate(
                        [jnp.where(sub_pc >= 4, vt[w0:w0 + 8], 1.0), vt[w0 + 8:w0 + 24]], axis=0)
                vt_ref[h, :, pl.ds(r0, PC)] = vw
            return carry

        lax.fori_loop(0, NPC, qv, 0)

        for cp in late_cp:
            cp.wait()

        def ffn(t, carry):
            r0 = pl.multiple_of(t * TR, TR)
            xn = xn_ref[pl.ds(r0, TR), :]
            y = x_ref[pl.ds(r0, TR), :].astype(f32)
            outs = []
            for c in range(F // FC):
                g = jnp.dot(xn, wg_ref[:, c * FC:(c + 1) * FC], preferred_element_type=f32)
                u = jnp.dot(xn, wu_ref[:, c * FC:(c + 1) * FC], preferred_element_type=f32)
                hh = (g * jax.nn.sigmoid(g) * u).astype(bf16)
                y = y + jnp.dot(hh, wd_ref[c * FC:(c + 1) * FC, :], preferred_element_type=f32)
                outs += [g, u]
            y_ref[pl.ds(r0, TR), :] = y
            nr = TR // 8
            nv = nr * (FC // 128)
            ppi = H // 2 // NR
            jobs = [(k, u, f0) for k in range(ppi) for u in range(KV // 8)
                    for f0 in range(0, 2 * DH, XP)]
            for n, (k, u, f0) in enumerate(jobs):
                pos = n * len(outs) * nv // len(jobs)
                r, col = pos % nr, (pos % nv) // nr
                tie = outs[pos // nv][8 * r:8 * r + 8, col * 128:(col + 1) * 128]
                pr = t * ppi + k
                kk = jnp.where(tie > 0.0, kf_ref[0, pr, 8 * u:8 * u + 8, :],
                               kf_ref[1, pr, 8 * u:8 * u + 8, :])
                for f in range(f0, f0 + XP):
                    kb_ref[pr, f, 8 * u:8 * u + 8, :] = jnp.broadcast_to(kk[:, f:f + 1], (8, 128))
            return carry

        lax.fori_loop(0, NR, ffn, 0)

        sub = lax.broadcasted_iota(jnp.int32, (8, TQ), 0)

        def load_qm(g, j, t0):
            lo, hi = DH * j, DH * j + DH
            rows = []
            for r in range(GW // 8):
                a, b = 8 * r, 8 * r + 8
                if b <= lo or a >= hi:
                    rows.append(None)
                    continue
                v = jnp.concatenate([qt_ref[g, t0 + t, a:b, :] for t in range(NT128)], axis=1)
                if a < lo:
                    v = jnp.where(sub >= lo - a, v, 0.0)
                elif b > hi:
                    v = jnp.where(sub < hi - a, v, 0.0)
                rows.append(v)
            rows.append(jnp.concatenate(
                [sh_ref[g * HPG + j, t0 + t] for t in range(NT128)], axis=1))
            rows += [None] * (16 - len(rows))
            blocks = []
            for r in range(8):
                a, b = rows[2 * r], rows[2 * r + 1]
                if a is None and b is None:
                    blocks.append(jnp.zeros((16, TQ), bf16))
                else:
                    a = jnp.zeros((8, TQ), f32) if a is None else a
                    b = jnp.zeros((8, TQ), f32) if b is None else b
                    blocks.append(jnp.concatenate([a, b], axis=0).astype(bf16))
            return jnp.concatenate(blocks, axis=0)

        def vpu_head(it, i, tok):
            ib = it // NQ
            t0 = (it % NQ) * NT128
            g, j = ib * GPI + i // HPG, i % HPG
            for t in range(NT128):
                qrow = [jnp.broadcast_to(qt_ref[g, t0 + t, j * DH + d:j * DH + d + 1, :], (8, 128))
                        for d in range(DH)]
                srow = [jnp.broadcast_to(sh_ref[g * HPG + j, t0 + t, r:r + 1, :], (8, 128))
                        for r in (3, 4)]
                for a in range(0, KV, 16):
                    init = srow[0] if tok is None else jnp.where(tok > 0.0, srow[0], srow[1])
                    acc = [init, init]
                    for d in range(DH):
                        for u in range(2):
                            acc[u] = acc[u] + qrow[d] * kb_ref[
                                ib * (NH // 2) + i // 2, (i % 2) * DH + d,
                                a + 8 * u:a + 8 * u + 8, :]
                    pk = pair_pack(jnp.exp2(jnp.concatenate(acc, axis=0)))
                    r0 = (KR + a) // 2
                    pl_ref[i, r0:r0 + 8, t * 128:(t + 1) * 128] = pk
                    tok = lax.bitcast_convert_type(pk, f32)
            return tok

        def attn_step(it, bad):
            g0 = (it // NQ) * GPI
            t0 = (it % NQ) * NT128
            q0 = pl.multiple_of((it % NQ) * TQ, TQ)
            qms = [None] * NH
            accs = [None] * NH
            nc = len(mchunks)
            steps = [(i, c) for i in range(NH) for c in range(nc)]
            tok = [None]
            zz = z_ref[0]

            def in_last_block(i, b):
                return b == KM and KR > 0 and i > 0

            def qk(n):
                i, c = steps[n]
                a, b = mchunks[c]
                g = g0 + i // HPG
                if qms[i] is None:
                    qms[i] = load_qm(g, i % HPG, t0)
                    if i + 1 < NH:
                        tok[0] = vpu_head(it, i + 1, tok[0])
                    else:
                        tok[0] = vpu_head((it + 1) % (NI * NQ), 0, tok[0])
                st = jnp.dot(k_ref[g, a:b, :], qms[i], preferred_element_type=f32)
                if in_last_block(i, b):
                    pl_ref[i, 0:(b - a) // 2, :] = pair_pack(jnp.exp2(st))
                else:
                    pbuf[n % NPB][zz, 0:(b - a) // 2, :] = pair_pack(jnp.exp2(st))

            def pv(i, a, b, pu):
                r = lax.dot_general(vt_ref[g0 * HPG + i, :, a:b], pltpu.bitcast(pu, bf16), NN,
                                    preferred_element_type=f32)
                accs[i] = r if accs[i] is None else accs[i] + r

            def finish(i, bad):
                outs = []
                for odd, a in enumerate((accs[i], accs[i + 1])):
                    lv = a[0:8] if odd else a[16:24]
                    keep = (sub < 4) if odd else (sub >= 4)
                    l = jnp.where(keep, lv, pltpu.roll(lv, 4, 0))
                    r = 1.0 / l
                    amax = jnp.maximum(jnp.maximum(jnp.abs(a[0:8]), jnp.abs(a[8:16])),
                                       jnp.abs(a[16:24]))
                    ok = (l >= L_MIN) & (amax <= ACC_MAX)
                    bad = jnp.where(ok, bad, 1.0)
                    outs.append([a[0:8] * r, a[8:16] * r, a[16:24] * r])
                mid = jnp.where(sub < 4, outs[0][2], outs[1][0])
                o = jnp.concatenate([outs[0][0], outs[0][1], mid, outs[1][1], outs[1][2]], axis=0)
                ot_ref[pl.ds(pl.multiple_of(g0 * GW + i * DH, 8), 40), pl.ds(q0, TQ)] = o
                return bad

            pv0 = pl_ref[0, KR // 2:, :]
            for n in range(DEPTH):
                qk(n)
            for n, (i, c) in enumerate(steps):
                a, b = mchunks[c]
                if n + DEPTH < len(steps):
                    qk(n + DEPTH)
                if not in_last_block(i, b):
                    pv(i, a, b, pbuf[n % NPB][zz, 0:(b - a) // 2, :])
                if i == 0 and c == 0:
                    pv(i, KM, S, pv0)
                if i > 0 and c == nc - 1:
                    pv(i, S - KL, S, pl_ref[i])
                if i % 2 == 1 and c == nc - 1:
                    bad = finish(i - 1, bad)
            return bad

        def true_max():
            rows80 = lax.broadcasted_iota(jnp.int32, (GW, TQ), 0)

            def one(it, carry):
                h = it // NQ
                t0 = (it % NQ) * NT128
                g = h // HPG
                lo = (h % HPG) * DH
                win = jnp.concatenate([qt_ref[g, t0 + t] for t in range(NT128)], axis=1)
                qm = jnp.concatenate(
                    [jnp.where((rows80 >= lo) & (rows80 < lo + DH), win, 0.0),
                     jnp.zeros((128 - GW, TQ), f32)], axis=0).astype(bf16)

                def chunk(c, mx):
                    st = jnp.dot(k_ref[g, pl.ds(pl.multiple_of(c * 256, 256), 256), :], qm,
                                 preferred_element_type=f32)
                    return jnp.maximum(mx, jnp.max(st, axis=0, keepdims=True))

                mx = lax.fori_loop(0, S // 256, chunk, jnp.full((1, TQ), -jnp.inf, f32))
                m1 = mx.astype(bf16).astype(f32)
                m2 = (mx - m1).astype(bf16).astype(f32)
                m3 = (mx - m1 - m2).astype(bf16).astype(f32)
                shv = jnp.where(sub == 0, -m1, jnp.where(sub == 1, -m2, jnp.where(
                    sub == 2, -m3, jnp.where((sub == 3) | (sub == 4), -(m1 + m2 + m3), 0.0))))
                for t in range(NT128):
                    sh_ref[h, t0 + t] = shv[:, t * 128:(t + 1) * 128]
                return carry

            lax.fori_loop(0, H * NQ, one, 0)

        def attempt(state):
            n, _ = state

            @pl.when(n > 0)
            def _():
                true_max()

            pl_ref[0, KR // 2:, :] = pair_pack(jnp.exp2(jnp.dot(
                k_ref[0, KM:S, :], load_qm(0, 0, 0), preferred_element_type=f32)))
            bad = lax.fori_loop(0, NI * NQ, attn_step, jnp.zeros((8, TQ), f32))
            unsafe = jnp.max(bad) > (-1.0 if FORCE_FALLBACK else 0.0)
            return n + 1, unsafe.astype(jnp.int32)

        lax.while_loop(lambda s: (s[0] < 2) & (s[1] > 0), attempt,
                       (jnp.int32(0), jnp.int32(1)))

        out_cp = [pltpu.make_async_copy(ob_ref.at[t * TO:(t + 1) * TO],
                                        o_hbm.at[t * TO:(t + 1) * TO], sem_o.at[t])
                  for t in range(S // TO)]
        for t in range(S // TO):
            a, b = t * TO, (t + 1) * TO
            y = y_ref[a:b, :] + lax.dot_general(ot_ref[:, a:b].astype(bf16), wo_ref[...], TN,
                                                preferred_element_type=f32)
            ob_ref[a:b, :] = y.astype(bf16)
            out_cp[t].start()
        for cp in out_cp:
            cp.wait()

    def run(A_x, A_wqkv, A_wo, B_x, B_w_gate, B_w_up, B_w_down):
        x = A_x.reshape(S, D)
        anyspec = pl.BlockSpec(memory_space=pl.ANY)
        out = pl.pallas_call(
            kernel,
            in_specs=[anyspec] * 6,
            out_specs=anyspec,
            out_shape=jax.ShapeDtypeStruct((S, D), bf16),
            scratch_shapes=[
                pltpu.VMEM((S, D), bf16),
                pltpu.VMEM((D, 3 * D), bf16),
                pltpu.VMEM((D, D), bf16),
                pltpu.VMEM((D, F), bf16),
                pltpu.VMEM((D, F), bf16),
                pltpu.VMEM((F, D), bf16),
                pltpu.VMEM((S, D), bf16),
                pltpu.VMEM((S, D), bf16),
                pltpu.VMEM((S // 2, D), u32),
                pltpu.VMEM((NG, S, 128), bf16),
                pltpu.VMEM((NG, S // 128, GW, 128), f32),
                pltpu.VMEM((H, S // 128, 8, 128), f32),
                pltpu.VMEM((H, 24, S), f32),
                pltpu.VMEM((2 * D, D), bf16),
                pltpu.VMEM((H, S), f32),
                pltpu.VMEM((D, S), f32),
                pltpu.VMEM((NH, KL // 2, TQ), u32),
                pltpu.VMEM((2, H // 2, KV, 128), f32),
                pltpu.VMEM((H // 2, 2 * DH, KV, 128), f32),
                pltpu.VMEM((S, D), f32),
                pltpu.SemaphoreType.DMA((len(blocks),)),
                pltpu.SemaphoreType.DMA((7,)),
                pltpu.SemaphoreType.DMA((S // TO,)),
                pltpu.SMEM((1,), jnp.int32),
            ] + [pltpu.VMEM((2, KC // 2, TQ), u32) for _ in range(NPB)],
            compiler_params=pltpu.CompilerParams(vmem_limit_bytes=126 * 1024 * 1024),
            interpret=INTERP,
        )(x, A_wqkv, A_wo, B_w_gate, B_w_up, B_w_down)
        return out.reshape(1, S, D)

    return run


_run = make_kernel()


@jax.jit
def pallas_parallel_sum__mha_block__swiglu_ffn__prompt_kernel(
    A_x: jax.Array,
    A_wqkv: jax.Array,
    A_wo: jax.Array,
    B_x: jax.Array,
    B_w_gate: jax.Array,
    B_w_up: jax.Array,
    B_w_down: jax.Array,
):
    return _run(A_x, A_wqkv, A_wo, B_x, B_w_gate, B_w_up, B_w_down)
```

```python
import math

import jax
import jax.numpy as jnp
from jax import lax
import jax.experimental.pallas as pl
import jax.experimental.pallas.tpu as pltpu

S, D, H, DH, F = 2048, 640, 32, 20, 1536
HPG = 4
NG = H // HPG
GW = HPG * DH
GPI = 2
NH = GPI * HPG
NI = NG // GPI
QSCALE = (DH ** -0.5) * math.log2(math.e)
M_OFFSET = 72.0
L_MIN = 2.0 ** -40
ACC_MAX = 2.0 ** 120

f32 = jnp.float32
bf16 = jnp.bfloat16
u32 = jnp.uint32
NT = (((1,), (1,)), ((), ()))
TN = (((0,), (0,)), ((), ()))
NN = (((1,), (0,)), ((), ()))

TQ = 512
NT128 = TQ // 128
NQ = S // TQ
PC = 512
NPC = S // PC


def make_kernel(KC=128, DEPTH=5, TR=256, FC=512, NPB=8, MS=64, KV=160, XP=10, TO=128,
                FORCE_FALLBACK=False, INTERP=False, BL=(512, 1536), SUB=512):
    NR = S // TR
    blocks = list(zip((0,) + tuple(BL), tuple(BL) + (S,)))
    KM = S - KV
    KL = -(-KV // 128) * 128
    KR = KL - KV
    mchunks = [(c, min(c + KC, S - KL)) for c in range(0, S - KL, KC)]
    if KR:
        mchunks.append((S - KL, KM))
    assert KV % 16 == 0 and KV > 0 and (2 * DH) % XP == 0 and (H // 2) % NR == 0

    def pair_pack(v, rnd=False):
        n, m = v.shape
        u = lax.bitcast_convert_type(v, u32)
        if rnd:
            u = u + jnp.uint32(0x8000)
        e = u.reshape(n // 16, 2, 8, m)
        lo = lax.shift_right_logical(e[:, 0].reshape(n // 2, m), jnp.uint32(16))
        hi = e[:, 1].reshape(n // 2, m) & jnp.uint32(0xFFFF0000)
        return lo | hi

    def kernel(x_hbm, wqkv_hbm, wo_hbm, wg_hbm, wu_hbm, wd_hbm, o_hbm,
               x_ref, wqkv_ref, wo_ref, wg_ref, wu_ref, wd_ref, ob_ref,
               xn_ref, xv_ref, k_ref, qt_ref, sh_ref, vt_ref, wqvt_ref, kn2_ref, ot_ref,
               pl_ref, kf_ref, kb_ref, y_ref, sem_x, sem_w, sem_o, z_ref, *pbuf):
        z_ref[0] = 0
        x_cp = [pltpu.make_async_copy(x_hbm.at[a:b], x_ref.at[a:b], sem_x.at[c])
                for c, (a, b) in enumerate(blocks)]
        wk_cp, wq_cp, wv_cp = [
            pltpu.make_async_copy(wqkv_hbm.at[:, a:a + D], wqkv_ref.at[:, a:a + D], sem_w.at[i])
            for i, a in enumerate((D, 0, 2 * D))]
        late_cp = [pltpu.make_async_copy(s, d, sem_w.at[3 + i]) for i, (s, d) in enumerate(
            [(wg_hbm, wg_ref), (wu_hbm, wu_ref), (wd_hbm, wd_ref), (wo_hbm, wo_ref)])]
        x_cp[0].start()
        wk_cp.start()
        for cp in x_cp[1:]:
            cp.start()
        wq_cp.start()
        wv_cp.start()

        def layernorm(a, b):
            x = x_ref[a:b, :].astype(f32)
            mu = jnp.mean(x, axis=-1, keepdims=True)
            xc = x - mu
            var = jnp.mean(xc * xc, axis=-1, keepdims=True)
            xnf = xc * lax.rsqrt(var + 1e-5)
            xn_ref[a:b, :] = xnf.astype(bf16)
            xv_ref[a // 2:b // 2, :] = pair_pack(xnf, True)

        er2 = lax.broadcasted_iota(jnp.int32, (H, D), 0)
        ec2 = lax.broadcasted_iota(jnp.int32, (H, D), 1)
        e2 = jnp.where((ec2 >= er2 * DH) & (ec2 < er2 * DH + DH), 1.0, 0.0).astype(bf16)
        def kproj(a, b):
            kconst = jnp.where(lax.broadcasted_iota(jnp.int32, (b - a, 128 - GW), 1) < 3, 1.0, 0.0)
            kall = jnp.concatenate([
                jnp.dot(xn_ref[m:m + MS, :], wqkv_ref[:, D:2 * D], preferred_element_type=f32)
                for m in range(a, b, MS)], axis=0)
            kn2_ref[:, a:b] = lax.dot_general(e2, (kall * kall).astype(bf16), NT,
                                              preferred_element_type=f32)
            for g in range(NG):
                k_ref[g, a:b, :] = jnp.concatenate(
                    [kall[:, g * GW:(g + 1) * GW], kconst], axis=1).astype(bf16)
            if b == S:
                kv = kall[b - a - KV:, :].astype(bf16).astype(f32)
                for pr in range(H // 2):
                    blk = jnp.concatenate([kv[:, 2 * DH * pr:2 * DH * (pr + 1)],
                                           jnp.zeros((KV, 128 - 2 * DH), f32)], axis=1)
                    kf_ref[0, pr] = blk
                    kf_ref[1, pr] = blk

        for c, (a, b) in enumerate(blocks):
            x_cp[c].wait()
            if c == 0:
                layernorm(a, b)
                wk_cp.wait()
                kproj(a, b)
                continue
            if c == len(blocks) - 1:
                wq_cp.wait()
                wv_cp.wait()
                for cp in late_cp:
                    cp.start()
            for m in range(a, b, SUB):
                layernorm(m, min(m + SUB, b))
                kproj(m, min(m + SUB, b))
        wqvt_ref[0:D, :] = wqkv_ref[:, 0:D].astype(f32).T.astype(bf16)
        wqvt_ref[D:2 * D, :] = wqkv_ref[:, 2 * D:3 * D].astype(f32).T.astype(bf16)

        kmax2 = jnp.max(kn2_ref[...], axis=-1, keepdims=True)

        sub_pc = lax.broadcasted_iota(jnp.int32, (8, PC), 0)

        def qv(c, carry):
            r0 = pl.multiple_of(c * PC, PC)
            xn = xn_ref[pl.ds(r0, PC), :]
            qt = lax.dot_general(wqvt_ref[0:D, :], xn, NT, preferred_element_type=f32)
            qt = (qt * QSCALE).astype(bf16).astype(f32)
            for t in range(PC // 128):
                for g in range(NG):
                    qt_ref[g, c * (PC // 128) + t] = qt[g * GW:(g + 1) * GW, t * 128:(t + 1) * 128]
            qn2 = jnp.dot(e2, (qt * qt).astype(bf16), preferred_element_type=f32)
            xv = pltpu.bitcast(
                xv_ref[pl.ds(pl.multiple_of(c * (PC // 2), PC // 2), PC // 2), :], bf16)
            vt = lax.dot_general(wqvt_ref[D:2 * D, :], xv, NT, preferred_element_type=f32)
            negm = M_OFFSET - jnp.sqrt(qn2 * kmax2) * (1.0 + 2.0 ** -6)
            negm = negm.astype(bf16).astype(f32)
            for h in range(H):
                shv = jnp.where((sub_pc == 0) | (sub_pc == 3) | (sub_pc == 4), negm[h:h + 1, :], 0.0)
                for t in range(PC // 128):
                    sh_ref[h, c * (PC // 128) + t] = shv[:, t * 128:(t + 1) * 128]
                w0 = 8 * ((DH * h) // 8)
                if h % 2 == 0:
                    vw = jnp.concatenate(
                        [vt[w0:w0 + 16], jnp.where(sub_pc < 4, vt[w0 + 16:w0 + 24], 1.0)], axis=0)
                else:
                    vw = jnp.concatenate(
                        [jnp.where(sub_pc >= 4, vt[w0:w0 + 8], 1.0), vt[w0 + 8:w0 + 24]], axis=0)
                vt_ref[h, :, pl.ds(r0, PC)] = vw
            return carry

        lax.fori_loop(0, NPC, qv, 0)

        for cp in late_cp:
            cp.wait()

        def ffn(t, carry):
            r0 = pl.multiple_of(t * TR, TR)
            xn = xn_ref[pl.ds(r0, TR), :]
            y = x_ref[pl.ds(r0, TR), :].astype(f32)
            outs = []
            for c in range(F // FC):
                g = jnp.dot(xn, wg_ref[:, c * FC:(c + 1) * FC], preferred_element_type=f32)
                u = jnp.dot(xn, wu_ref[:, c * FC:(c + 1) * FC], preferred_element_type=f32)
                hh = (g * jax.nn.sigmoid(g) * u).astype(bf16)
                y = y + jnp.dot(hh, wd_ref[c * FC:(c + 1) * FC, :], preferred_element_type=f32)
                outs += [g, u]
            y_ref[pl.ds(r0, TR), :] = y
            nr = TR // 8
            nv = nr * (FC // 128)
            ppi = H // 2 // NR
            jobs = [(k, u, f0) for k in range(ppi) for u in range(KV // 8)
                    for f0 in range(0, 2 * DH, XP)]
            for n, (k, u, f0) in enumerate(jobs):
                pos = n * len(outs) * nv // len(jobs)
                r, col = pos % nr, (pos % nv) // nr
                tie = outs[pos // nv][8 * r:8 * r + 8, col * 128:(col + 1) * 128]
                pr = t * ppi + k
                kk = jnp.where(tie > 0.0, kf_ref[0, pr, 8 * u:8 * u + 8, :],
                               kf_ref[1, pr, 8 * u:8 * u + 8, :])
                kb_ref[pr, f0:f0 + XP, 8 * u:8 * u + 8, :] = jnp.stack(
                    [jnp.broadcast_to(kk[:, f:f + 1], (8, 128)) for f in range(f0, f0 + XP)])
            return carry

        lax.fori_loop(0, NR, ffn, 0)

        sub = lax.broadcasted_iota(jnp.int32, (8, TQ), 0)

        def load_qm(g, j, t0):
            lo, hi = DH * j, DH * j + DH
            rows = []
            for r in range(GW // 8):
                a, b = 8 * r, 8 * r + 8
                if b <= lo or a >= hi:
                    rows.append(None)
                    continue
                v = jnp.concatenate([qt_ref[g, t0 + t, a:b, :] for t in range(NT128)], axis=1)
                if a < lo:
                    v = jnp.where(sub >= lo - a, v, 0.0)
                elif b > hi:
                    v = jnp.where(sub < hi - a, v, 0.0)
                rows.append(v)
            rows.append(jnp.concatenate(
                [sh_ref[g * HPG + j, t0 + t] for t in range(NT128)], axis=1))
            rows += [None] * (16 - len(rows))
            blocks = []
            for r in range(8):
                a, b = rows[2 * r], rows[2 * r + 1]
                if a is None and b is None:
                    blocks.append(jnp.zeros((16, TQ), bf16))
                else:
                    a = jnp.zeros((8, TQ), f32) if a is None else a
                    b = jnp.zeros((8, TQ), f32) if b is None else b
                    blocks.append(jnp.concatenate([a, b], axis=0).astype(bf16))
            return jnp.concatenate(blocks, axis=0)

        def vpu_head(it, i, tok):
            ib = it // NQ
            t0 = (it % NQ) * NT128
            g, j = ib * GPI + i // HPG, i % HPG
            pair, f0 = ib * (NH // 2) + i // 2, (i % 2) * DH
            for t in range(NT128):
                qrow = [jnp.broadcast_to(qt_ref[g, t0 + t, j * DH + d:j * DH + d + 1, :], (8, 128))
                        for d in range(DH)]
                qrow = [jnp.concatenate([q, q], axis=0) for q in qrow]
                srow = [jnp.broadcast_to(sh_ref[g * HPG + j, t0 + t, r:r + 1, :], (8, 128))
                        for r in (3, 4)]
                for a in range(0, KV, 16):
                    init = srow[0] if tok is None else jnp.where(tok > 0.0, srow[0], srow[1])
                    acc = jnp.concatenate([init, init], axis=0)
                    for d in range(DH):
                        acc = acc + qrow[d] * kb_ref[pair, f0 + d, a:a + 16, :]
                    pk = pair_pack(jnp.exp2(acc))
                    r0 = (KR + a) // 2
                    pl_ref[i, r0:r0 + 8, t * 128:(t + 1) * 128] = pk
                    tok = lax.bitcast_convert_type(pk, f32)
            return tok

        def attn_step(it, bad):
            g0 = (it // NQ) * GPI
            t0 = (it % NQ) * NT128
            q0 = pl.multiple_of((it % NQ) * TQ, TQ)
            qms = [None] * NH
            accs = [None] * NH
            nc = len(mchunks)
            steps = [(i, c) for i in range(NH) for c in range(nc)]
            tok = [None]
            zz = z_ref[0]

            def in_last_block(i, b):
                return b == KM and KR > 0 and i > 0

            def qk(n):
                i, c = steps[n]
                a, b = mchunks[c]
                g = g0 + i // HPG
                if qms[i] is None:
                    qms[i] = load_qm(g, i % HPG, t0)
                    if i + 1 < NH:
                        tok[0] = vpu_head(it, i + 1, tok[0])
                    else:
                        tok[0] = vpu_head((it + 1) % (NI * NQ), 0, tok[0])
                st = jnp.dot(k_ref[g, a:b, :], qms[i], preferred_element_type=f32)
                if in_last_block(i, b):
                    pl_ref[i, 0:(b - a) // 2, :] = pair_pack(jnp.exp2(st))
                else:
                    pbuf[n % NPB][zz, 0:(b - a) // 2, :] = pair_pack(jnp.exp2(st))

            def pv(i, a, b, pu):
                r = lax.dot_general(vt_ref[g0 * HPG + i, :, a:b], pltpu.bitcast(pu, bf16), NN,
                                    preferred_element_type=f32)
                accs[i] = r if accs[i] is None else accs[i] + r

            def finish(i, bad):
                outs = []
                for odd, a in enumerate((accs[i], accs[i + 1])):
                    lv = a[0:8] if odd else a[16:24]
                    keep = (sub < 4) if odd else (sub >= 4)
                    l = jnp.where(keep, lv, pltpu.roll(lv, 4, 0))
                    r = 1.0 / l
                    amax = jnp.maximum(jnp.maximum(jnp.abs(a[0:8]), jnp.abs(a[8:16])),
                                       jnp.abs(a[16:24]))
                    ok = (l >= L_MIN) & (amax <= ACC_MAX)
                    bad = jnp.where(ok, bad, 1.0)
                    outs.append([a[0:8] * r, a[8:16] * r, a[16:24] * r])
                mid = jnp.where(sub < 4, outs[0][2], outs[1][0])
                o = jnp.concatenate([outs[0][0], outs[0][1], mid, outs[1][1], outs[1][2]], axis=0)
                ot_ref[pl.ds(pl.multiple_of(g0 * GW + i * DH, 8), 40), pl.ds(q0, TQ)] = o
                return bad

            pv0 = pl_ref[0, KR // 2:, :]
            for n in range(DEPTH):
                qk(n)
            for n, (i, c) in enumerate(steps):
                a, b = mchunks[c]
                if n + DEPTH < len(steps):
                    qk(n + DEPTH)
                if not in_last_block(i, b):
                    pv(i, a, b, pbuf[n % NPB][zz, 0:(b - a) // 2, :])
                if i == 0 and c == 0:
                    pv(i, KM, S, pv0)
                if i > 0 and c == nc - 1:
                    pv(i, S - KL, S, pl_ref[i])
                if i % 2 == 1 and c == nc - 1:
                    bad = finish(i - 1, bad)
            return bad

        def true_max():
            rows80 = lax.broadcasted_iota(jnp.int32, (GW, TQ), 0)

            def one(it, carry):
                h = it // NQ
                t0 = (it % NQ) * NT128
                g = h // HPG
                lo = (h % HPG) * DH
                win = jnp.concatenate([qt_ref[g, t0 + t] for t in range(NT128)], axis=1)
                qm = jnp.concatenate(
                    [jnp.where((rows80 >= lo) & (rows80 < lo + DH), win, 0.0),
                     jnp.zeros((128 - GW, TQ), f32)], axis=0).astype(bf16)

                def chunk(c, mx):
                    st = jnp.dot(k_ref[g, pl.ds(pl.multiple_of(c * 256, 256), 256), :], qm,
                                 preferred_element_type=f32)
                    return jnp.maximum(mx, jnp.max(st, axis=0, keepdims=True))

                mx = lax.fori_loop(0, S // 256, chunk, jnp.full((1, TQ), -jnp.inf, f32))
                m1 = mx.astype(bf16).astype(f32)
                m2 = (mx - m1).astype(bf16).astype(f32)
                m3 = (mx - m1 - m2).astype(bf16).astype(f32)
                shv = jnp.where(sub == 0, -m1, jnp.where(sub == 1, -m2, jnp.where(
                    sub == 2, -m3, jnp.where((sub == 3) | (sub == 4), -(m1 + m2 + m3), 0.0))))
                for t in range(NT128):
                    sh_ref[h, t0 + t] = shv[:, t * 128:(t + 1) * 128]
                return carry

            lax.fori_loop(0, H * NQ, one, 0)

        def attempt(state):
            n, _ = state

            @pl.when(n > 0)
            def _():
                true_max()

            pl_ref[0, KR // 2:, :] = pair_pack(jnp.exp2(jnp.dot(
                k_ref[0, KM:S, :], load_qm(0, 0, 0), preferred_element_type=f32)))
            bad = lax.fori_loop(0, NI * NQ, attn_step, jnp.zeros((8, TQ), f32))
            unsafe = jnp.max(bad) > (-1.0 if FORCE_FALLBACK else 0.0)
            return n + 1, unsafe.astype(jnp.int32)

        lax.while_loop(lambda s: (s[0] < 2) & (s[1] > 0), attempt,
                       (jnp.int32(0), jnp.int32(1)))

        out_cp = [pltpu.make_async_copy(ob_ref.at[t * TO:(t + 1) * TO],
                                        o_hbm.at[t * TO:(t + 1) * TO], sem_o.at[t])
                  for t in range(S // TO)]
        for t in range(S // TO):
            a, b = t * TO, (t + 1) * TO
            y = y_ref[a:b, :] + lax.dot_general(ot_ref[:, a:b].astype(bf16), wo_ref[...], TN,
                                                preferred_element_type=f32)
            ob_ref[a:b, :] = y.astype(bf16)
            out_cp[t].start()
        for cp in out_cp:
            cp.wait()

    def run(A_x, A_wqkv, A_wo, B_x, B_w_gate, B_w_up, B_w_down):
        x = A_x.reshape(S, D)
        anyspec = pl.BlockSpec(memory_space=pl.ANY)
        out = pl.pallas_call(
            kernel,
            in_specs=[anyspec] * 6,
            out_specs=anyspec,
            out_shape=jax.ShapeDtypeStruct((S, D), bf16),
            scratch_shapes=[
                pltpu.VMEM((S, D), bf16),
                pltpu.VMEM((D, 3 * D), bf16),
                pltpu.VMEM((D, D), bf16),
                pltpu.VMEM((D, F), bf16),
                pltpu.VMEM((D, F), bf16),
                pltpu.VMEM((F, D), bf16),
                pltpu.VMEM((S, D), bf16),
                pltpu.VMEM((S, D), bf16),
                pltpu.VMEM((S // 2, D), u32),
                pltpu.VMEM((NG, S, 128), bf16),
                pltpu.VMEM((NG, S // 128, GW, 128), f32),
                pltpu.VMEM((H, S // 128, 8, 128), f32),
                pltpu.VMEM((H, 24, S), f32),
                pltpu.VMEM((2 * D, D), bf16),
                pltpu.VMEM((H, S), f32),
                pltpu.VMEM((D, S), f32),
                pltpu.VMEM((NH, KL // 2, TQ), u32),
                pltpu.VMEM((2, H // 2, KV, 128), f32),
                pltpu.VMEM((H // 2, 2 * DH, KV, 128), f32),
                pltpu.VMEM((S, D), f32),
                pltpu.SemaphoreType.DMA((len(blocks),)),
                pltpu.SemaphoreType.DMA((7,)),
                pltpu.SemaphoreType.DMA((S // TO,)),
                pltpu.SMEM((1,), jnp.int32),
            ] + [pltpu.VMEM((2, KC // 2, TQ), u32) for _ in range(NPB)],
            compiler_params=pltpu.CompilerParams(vmem_limit_bytes=126 * 1024 * 1024),
            interpret=INTERP,
        )(x, A_wqkv, A_wo, B_w_gate, B_w_up, B_w_down)
        return out.reshape(1, S, D)

    return run


_run = make_kernel()


@jax.jit
def pallas_parallel_sum__mha_block__swiglu_ffn__prompt_kernel(
    A_x: jax.Array,
    A_wqkv: jax.Array,
    A_wo: jax.Array,
    B_x: jax.Array,
    B_w_gate: jax.Array,
    B_w_up: jax.Array,
    B_w_down: jax.Array,
):
    return _run(A_x, A_wqkv, A_wo, B_x, B_w_gate, B_w_up, B_w_down)
```
